```python
import jax
import jax.numpy as jnp

def _softmax(x, axis=-1):
    return jax.nn.softmax(x, axis=axis)

def _gelu(x):
    return jax.nn.gelu(x, approximate=True)

def _silu(x):
    return jax.nn.silu(x)

def _sigmoid(x):
    return jax.nn.sigmoid(x)

def _layernorm(x, axis=-1, eps=1e-05):
    m = jnp.mean(x, axis=axis, keepdims=True)
    v = jnp.var(x, axis=axis, keepdims=True)
    return (x - m) / jnp.sqrt(v + eps)

def _scatter_add(tgt, idx, src, axis=0):
    return tgt.at[idx].add(src)

def _segment_sum(src, seg, n):
    return jax.ops.segment_sum(src, seg, n)

class _Rng:

    def __init__(self, key):
        self._k = key

    def _next(self):
        self._k, sub = jax.random.split(self._k)
        return sub

    def normal(self, shape):
        return jax.random.normal(self._next(), shape, dtype=jnp.bfloat16)

    def randint(self, lo, hi, shape):
        return jax.random.randint(self._next(), shape, lo, hi, dtype=jnp.int32)

    def uniform(self, shape, lo=0.0, hi=1.0):
        return jax.random.uniform(self._next(), shape, jnp.bfloat16, lo, hi)

    def permutation(self, n):
        return jax.random.permutation(self._next(), n)
kernel_name = 'concat_heads__spectral_gfnet__memory_aug_recurrent_mem_tr__prompt'

def setup_inputs():
    _rng = _Rng(jax.random.key(int.from_bytes(__import__("os").urandom(4), "little")))
    _w = lambda a: (lambda t: t.astype(jnp.bfloat16) if jnp.issubdtype(t.dtype, jnp.floating) else t)(jnp.asarray(a))

    def _A_setup():
        B, S, D = (1, 2048, 1024)
        Df = D // 2 + 1
        return {'x': _w((lambda *s: _rng.normal(s) * 0.05)(B, S, D)), 'w_r': _w((lambda *s: _rng.normal(s) * 0.05)(S, Df) * 0.02), 'w_i': _w((lambda *s: _rng.normal(s) * 0.05)(S, Df) * 0.02)}
    _A_in = _A_setup()

    def _B_setup():
        B, S, Dm = (1, 2048, 1024)
        H, Dh = (32, 128)
        M, seg = (8, 32)
        seg = min(seg, S)
        S = S // seg * seg
        return {'x': _w((lambda *s: _rng.normal(s) * 0.05)(B, S, Dm)), 'mem0': _w((lambda *s: _rng.normal(s) * 0.05)(B, M, Dm)), 'Wq': _w((lambda *s: _rng.normal(s) * 0.05)(Dm, H, Dh) * Dm ** (-0.5)), 'Wk': _w((lambda *s: _rng.normal(s) * 0.05)(Dm, H, Dh) * Dm ** (-0.5)), 'Wv': _w((lambda *s: _rng.normal(s) * 0.05)(Dm, H, Dh) * Dm ** (-0.5)), 'Wo': _w((lambda *s: _rng.normal(s) * 0.05)(H, Dh, Dm) * (H * Dh) ** (-0.5)), 'seg_len': seg}
    _B_in = _B_setup()
    return {'A_x': _A_in['x'], 'A_w_r': _A_in['w_r'], 'A_w_i': _A_in['w_i'], 'B_x': _B_in['x'], 'B_mem0': _B_in['mem0'], 'B_Wq': _B_in['Wq'], 'B_Wk': _B_in['Wk'], 'B_Wv': _B_in['Wv'], 'B_Wo': _B_in['Wo'], 'B_seg_len': _B_in['seg_len']}

def reference(A_x, A_w_r, A_w_i, B_x, B_mem0, B_Wq, B_Wk, B_Wv, B_Wo, B_seg_len):

    def _A_ref(x, w_r, w_i):
        B, S, D = x.shape
        X = (lambda x, axes=(-2, -1): jnp.fft.rfft2(x.astype(jnp.float32), axes=axes))(x, axes=(-2, -1))
        W = w_r + 1j * w_i
        X = X * W
        y = (lambda x, s, axes=(-2, -1): jnp.fft.irfft2(x, s=s, axes=axes).astype(jnp.bfloat16))(X, (S, D), axes=(-2, -1))
        return y

    def _B_ref(x, mem0, Wq, Wk, Wv, Wo, seg_len):
        B, S, Dm = x.shape
        H, Dh = (Wq.shape[1], Wq.shape[2])
        M = mem0.shape[1]
        scale = Dh ** (-0.5)
        n_seg = S // seg_len
        L = M + seg_len
        idx = jnp.arange(L)
        mask = (idx[:, None] < M) | (idx[:, None] >= idx[None, :])
        mem = mem0
        outs = []
        for s in range(n_seg):
            xs = x[:, s * seg_len:(s + 1) * seg_len, :].copy()
            h = jnp.concatenate([mem, xs], axis=1)
            q = jnp.einsum('btd,dhe->bhte', h, Wq)
            k = jnp.einsum('btd,dhe->bhte', h, Wk)
            v = jnp.einsum('btd,dhe->bhte', h, Wv)
            scores = jnp.einsum('bhqe,bhke->bhqk', q, k) * scale
            scores = jnp.where(mask[None, None], scores, -1000000000.0)
            p = _softmax(scores, axis=-1)
            o = jnp.einsum('bhqk,bhke->bhqe', p, v)
            o = jnp.einsum('bhte,hed->btd', o, Wo)
            mem = o[:, :M, :].copy()
            outs.append(o[:, M:, :])
        return jnp.concatenate(outs, axis=1)
    a = _A_ref(A_x, A_w_r, A_w_i)
    b = _B_ref(B_x, B_mem0, B_Wq, B_Wk, B_Wv, B_Wo, B_seg_len)
    return jnp.concatenate([a, b], axis=-1)
```

```python
import functools
import math

import jax
import jax.numpy as jnp
from jax import lax
import jax.experimental.pallas as pl
import jax.experimental.pallas.tpu as pltpu

bf16, f32, i32 = jnp.bfloat16, jnp.float32, jnp.int32

S, D = 2048, 1024
H, DH = 32, 128
M, SEG = 8, 32
L = M + SEG
NSEG = S // SEG
XCHUNK = 256
NXCHUNK = S // XCHUNK

_NN = (((1,), (0,)), ((), ()))
_NT = (((1,), (1,)), ((), ()))
_HI16 = -65536
_R2 = math.sqrt(0.5)
_SCALE = 2.0 ** -5


def _dot(a, b, dims=_NN):
    return lax.dot_general(a, b, dims, preferred_element_type=f32)


def _lo_f32(w):
    return pltpu.bitcast(w << 16, f32)


def _hi_f32(w):
    return pltpu.bitcast(w & _HI16, f32)


def _cadd(a, b):
    return a[0] + b[0], a[1] + b[1]


def _csub(a, b):
    return a[0] - b[0], a[1] - b[1]


def _fft4(x0, x1, x2, x3, sign):
    a, b = _cadd(x0, x2), _csub(x0, x2)
    c, d = _cadd(x1, x3), _csub(x1, x3)
    minus_i = (b[0] + d[1], b[1] - d[0])
    plus_i = (b[0] - d[1], b[1] + d[0])
    if sign < 0:
        return _cadd(a, c), minus_i, _csub(a, c), plus_i
    return _cadd(a, c), plus_i, _csub(a, c), minus_i


def _twiddle16(x, m, sign):
    if m == 0:
        return x
    if m == 4:
        return (-x[1], x[0]) if sign > 0 else (x[1], -x[0])
    if m == 2:
        if sign > 0:
            return (x[0] - x[1]) * _R2, (x[0] + x[1]) * _R2
        return (x[0] + x[1]) * _R2, (x[1] - x[0]) * _R2
    if m == 6:
        if sign > 0:
            return (x[0] + x[1]) * -_R2, (x[0] - x[1]) * _R2
        return (x[1] - x[0]) * _R2, (x[0] + x[1]) * -_R2
    c, s = math.cos(2 * math.pi * m / 16), sign * math.sin(2 * math.pi * m / 16)
    return x[0] * c - x[1] * s, x[0] * s + x[1] * c


def _fft16(x, sign):
    t = [None] * 16
    for a0 in range(4):
        ys = _fft4(x[a0], x[4 + a0], x[8 + a0], x[12 + a0], sign)
        for k0 in range(4):
            t[4 * a0 + k0] = _twiddle16(ys[k0], a0 * k0, sign)
    y = [None] * 16
    for k0 in range(4):
        ys = _fft4(t[k0], t[4 + k0], t[8 + k0], t[12 + k0], sign)
        for k1 in range(4):
            y[k0 + 4 * k1] = ys[k1]
    return y


def _rfft8(x):
    s04, d04 = x[0] + x[4], x[0] - x[4]
    s26, d26 = x[2] + x[6], x[2] - x[6]
    s15, d15 = x[1] + x[5], x[1] - x[5]
    s37, d37 = x[3] + x[7], x[3] - x[7]
    e, o = s04 + s26, s15 + s37
    p, q = (d15 - d37) * _R2, (d15 + d37) * _R2
    return (e + o, e - o), (d04 + p, -(d26 + q)), (s04 - s26, s37 - s15), (d04 - p, d26 - q)


def _irfft8(r0, r1, r2, r3):
    a0, a4 = r0[0] + r0[1], r0[0] - r0[1]
    e0, e2 = a0 + r2[0], a0 - r2[0]
    e1, e3 = a4 - r2[1], a4 + r2[1]
    o0, o2 = r1[0] + r3[0], r3[1] - r1[1]
    dr, si = r1[0] - r3[0], r1[1] + r3[1]
    o1, o3 = (dr - si) * _R2, (dr + si) * -_R2
    return [e0 + o0, e1 + o1, e2 + o2, e3 + o3, e0 - o0, e1 - o1, e2 - o2, e3 - o3]


def _build_dft_matrices(m1, m2):
    ri = lax.broadcasted_iota(i32, (128, 128), 0)
    ci = lax.broadcasted_iota(i32, (128, 128), 1)
    ang = ((ri * ci) & 127).astype(f32) * (2 * math.pi / 128)
    cb, sb = jnp.cos(ang), jnp.sin(ang)
    ang = (ri[0:16] * ci[0:16]).astype(f32) * (2 * math.pi / S)
    ct_all, st_all = jnp.cos(ang) * _SCALE, jnp.sin(ang) * _SCALE

    def rotated(rows, a):
        ct, st = ct_all[a:a + 1], st_all[a:a + 1]
        return cb[0:rows] * ct - sb[0:rows] * st, sb[0:rows] * ct + cb[0:rows] * st

    for a in range(16):
        c, s = rotated(128, a)
        m2[a, 0:128, 0:128] = c.astype(bf16)
        m2[a, 0:128, 128:256] = (-s).astype(bf16)
        m2[a, 128:256, 0:128] = s.astype(bf16)
        m2[a, 128:256, 128:256] = c.astype(bf16)
    zero = jnp.zeros((64, 128), f32)
    for p in range(4):
        c0, s0 = rotated(64, 2 * p)
        c1, s1 = rotated(64, 2 * (4 if p == 0 else 8 - p))
        if p == 0:
            nyquist = jnp.where((ci[0:64] & 1) == 0, _SCALE, -_SCALE)
            blocks = [[c0, zero], [zero, c1],
                      [jnp.where(ri[0:64] == 0, nyquist, -s0), zero], [zero, -s1]]
        else:
            blocks = [[c0, s0], [c1, -s1], [-s0, c0], [-s1, -c1]]
        for i, (left, right) in enumerate(blocks):
            m1[p, i * 64:(i + 1) * 64, 0:128] = left.astype(bf16)
            m1[p, i * 64:(i + 1) * 64, 128:256] = right.astype(bf16)


def _forward_tiles(r, xv, m1, m2, gbuf):
    sub = lax.broadcasted_iota(i32, (8, 128), 0)
    for e, extract in enumerate((_lo_f32, _hi_f32)):
        a = 2 * r + e
        u = _rfft8([extract(xv[r, :, j * 128:(j + 1) * 128]) for j in range(8)])
        m2a = m2[a]
        for p in range(4):
            ab = jnp.concatenate([u[p][0].astype(bf16), u[p][1].astype(bf16)], axis=1)
            t = _dot(m1[p], ab, _NT)
            tr, ti = t[0:128], t[128:256]
            if p == 0:
                nyq = jnp.where(sub == 0, ti[0:8], 0.0)
                ti = jnp.concatenate([jnp.where(sub == 0, 0.0, ti[0:8]), ti[8:128],
                                      jnp.zeros((8, 128), f32)], axis=0)
                tr = jnp.concatenate([tr, nyq], axis=0)
            g = _dot(jnp.concatenate([tr, ti], axis=1), m2a)
            for blk in range(16):
                gbuf[p * 16 + blk, a] = g[blk * 8:(blk + 1) * 8]
            if p == 0:
                gbuf[64, a] = g[128:136]


def _filter_rows(g, gbuf, filt):
    xs = _fft16([(gbuf[g, a, :, 0:128], gbuf[g, a, :, 128:256]) for a in range(16)], -1)
    ys = []
    for k1 in range(16):
        wr, wi = filt(k1)
        xr, xi = xs[k1]
        ys.append((xr * wr - xi * wi, xr * wi + xi * wr))
    hs = _fft16(ys, +1)
    for a in range(16):
        gbuf[g, a, :, 0:128] = hs[a][0]
        gbuf[g, a, :, 128:256] = hs[a][1]


def _inverse_tiles(r, m1, m2, gbuf, yv):
    lane = lax.broadcasted_iota(i32, (128, 128), 1)
    ys = []
    for e in range(2):
        a = 2 * r + e
        m2a = m2[a]
        rr = []
        for p in range(4):
            h = gbuf[p * 16:(p + 1) * 16, a].reshape(128, 256).astype(bf16)
            z = _dot(m2a, h, _NT)
            zr, zi = z[0:128], z[128:256]
            if p == 0:
                nyq = _dot(m2a[0:128], gbuf[64, a].astype(bf16), _NT)
                zi = jnp.where(lane == 0, nyq[:, 0:1], zi)
            v = _dot(jnp.concatenate([zr, zi], axis=1), m1[p])
            rr.append((v[:, 0:128], v[:, 128:256]))
        ys.append(_irfft8(*rr))
    for j in range(8):
        even = pltpu.bitcast(ys[0][j].astype(bf16).astype(f32), i32)
        odd = pltpu.bitcast(ys[1][j].astype(bf16).astype(f32), i32)
        yv[r, :, j * 128:(j + 1) * 128] = lax.shift_right_logical(even, 16) | odd


def _interleave_heads(wqkv, m, j):
    even, odd = wqkv[m, j, :, 0], wqkv[m, j, :, 1]
    wqkv[m, j, :, 0] = (even & 0xFFFF) | (odd << 16)
    wqkv[m, j, :, 1] = lax.shift_right_logical(even, 16) | (odd & _HI16)


def _segment(s, wqkv, wo32, xs, h_ref, outs):
    r0 = pl.multiple_of(s * SEG, SEG)
    h_ref[M:L, :] = xs[pl.ds(r0, SEG), :].astype(f32)
    row = lax.broadcasted_iota(i32, (L, L), 0)
    col = lax.broadcasted_iota(i32, (L, L), 1)
    mask = (row < M) | (row >= col)

    def project(h):
        ws = [pltpu.bitcast(wqkv[m, h // 2, :, h % 2].reshape(D // 2, DH), bf16) for m in range(3)]
        return [_dot(h_ref[...], w) for w in ws]

    def probabilities(q, k):
        sc = _dot(q, k.astype(bf16), _NT) * DH ** -0.5
        sc = jnp.where(mask, sc, -1e9)
        e = jnp.exp(sc - jnp.max(sc, axis=-1, keepdims=True))
        return e * pltpu.reciprocal(jnp.sum(e, axis=-1, keepdims=True), approx=False)

    def out_proj(o, n, lo, hi):
        w = pltpu.bitcast(wo32[n, lo * DH // 2:hi * DH // 2, :], bf16)
        return _dot(jnp.concatenate(o[lo:hi], axis=1), w)

    lag_scores, lag_mix, split = 2, 4, 24
    state, o, part = {}, [None] * H, [None] * 8
    for t in range(H + 8):
        if t < H:
            state[t] = project(t)
        else:
            part[t - H] = out_proj(o, t - H, 0, split)
        if 0 <= t - lag_scores < H:
            q, k, v = state[t - lag_scores]
            state[t - lag_scores] = (probabilities(q, k), v)
        if 0 <= t - lag_mix < H:
            p, v = state.pop(t - lag_mix)
            o[t - lag_mix] = _dot(p, v.astype(bf16))
    for n in range(8):
        res = out_proj(o, n, split, H) + part[n]
        h_ref[0:M, n * 128:(n + 1) * 128] = res[0:M]
        outs[pl.ds(r0, SEG), n * 128:(n + 1) * 128] = res[M:L].astype(bf16)


def _kernel(ax_hbm, wr_hbm, wi_hbm, bx_hbm, mem0_ref, wq_hbm, wk_hbm, wv_hbm, wo_hbm, out_hbm,
            xv, wrv, wiv, wnr, wni, m1, m2, gbuf, yv,
            wqkv, wo, xs, h_ref, outs,
            sem_ax, sem_f, sem_w, sem_wo, sem_bx, sem_ya, sem_yb):
    ax32 = ax_hbm.bitcast(i32)
    out32 = out_hbm.bitcast(i32)

    def ax_copy(r):
        return pltpu.make_async_copy(ax32.at[:, r, :], xv.at[r], sem_ax.at[r])

    def ya_copy(r):
        return pltpu.make_async_copy(yv.at[r], out32.at[:, r, pl.ds(0, D)], sem_ya.at[0])

    def w_copies(m, j):
        w32 = (wq_hbm, wk_hbm, wv_hbm)[m].bitcast(i32)
        return [pltpu.make_async_copy(w32.at[:, :, e, j, :], wqkv.at[m, j, :, e],
                                      sem_w.at[m * (H // 2) + j]) for e in range(2)]

    def bx_copy(c):
        r0 = pl.multiple_of(c * XCHUNK, XCHUNK)
        return pltpu.make_async_copy(bx_hbm.at[pl.ds(r0, XCHUNK)], xs.at[pl.ds(r0, XCHUNK)],
                                     sem_bx.at[c])

    def yb_copies(s):
        return [pltpu.make_async_copy(outs.at[pl.ds(pl.multiple_of(s * SEG + 16 * i, 16), 16)],
                                      out_hbm.at[2 * s + i, :, pl.ds(D, D)], sem_yb.at[0])
                for i in range(SEG // 16)]

    f_copies = [pltpu.make_async_copy(src.at[pl.ds(0, D // 2), pl.ds(k1 * 128, 128)],
                                      dst.at[k1].bitcast(bf16), sem_f.at[0])
                for k1 in range(16) for src, dst in ((wr_hbm, wrv), (wi_hbm, wiv))]
    f_copies += [pltpu.make_async_copy(src.at[pl.ds(D // 2, 1), :], dst, sem_f.at[0])
                 for src, dst in ((wr_hbm, wnr), (wi_hbm, wni))]
    wo_copies = [pltpu.make_async_copy(wo_hbm.at[:, pl.ds(n * 128, 128)], wo.at[n], sem_wo.at[0])
                 for n in range(8)]

    for r in range(8):
        ax_copy(r).start()
    for cp in f_copies:
        cp.start()
    for m in range(3):
        for j in range(H // 2):
            for cp in w_copies(m, j):
                cp.start()
    bx_copy(0).start()
    for cp in wo_copies:
        cp.start()
    for c in range(1, NXCHUNK):
        bx_copy(c).start()

    _build_dft_matrices(m1, m2)

    @pl.loop(0, 8)
    def _(r):
        ax_copy(r).wait()
        _forward_tiles(r, xv, m1, m2, gbuf)

    for cp in f_copies:
        cp.wait()
    sub = lax.broadcasted_iota(i32, (8, 128), 0)

    @pl.loop(0, 64)
    def _(g):
        p, j = g // 16, g % 16
        k1d = jnp.where(j < 8, p, jnp.where(p == 0, 4, 8 - p))
        row0 = (k1d >> 1) + 32 * (j % 8)
        shift = 16 - 16 * (k1d & 1)
        half = jnp.where((sub == 0) & (g == 0), 0.5, 1.0)
        _filter_rows(g, gbuf, lambda k1: tuple(
            _hi_f32(w[k1, pl.ds(row0, 8, stride=4), :] << shift) * half for w in (wrv, wiv)))

    _filter_rows(64, gbuf, lambda k1: tuple(
        jnp.broadcast_to(w[:, k1 * 128:(k1 + 1) * 128].astype(f32) * 0.5, (8, 128))
        for w in (wnr, wni)))

    @pl.loop(0, 8)
    def _(r):
        _inverse_tiles(r, m1, m2, gbuf, yv)

    for m in range(3):
        @pl.loop(0, H // 2)
        def _(j, m=m):
            for cp in w_copies(m, j):
                cp.wait()
            _interleave_heads(wqkv, m, j)

    for cp in wo_copies:
        cp.wait()
    for r in range(8):
        ya_copy(r).start()
    h_ref[0:M, :] = mem0_ref[...].astype(f32)
    wo32 = wo.bitcast(i32)

    @pl.loop(0, NXCHUNK)
    def _(c):
        bx_copy(c).wait()

        @pl.loop(0, XCHUNK // SEG)
        def _(i):
            s = c * (XCHUNK // SEG) + i
            _segment(s, wqkv, wo32, xs, h_ref, outs)
            for cp in yb_copies(s):
                cp.start()

    for r in range(8):
        ya_copy(r).wait()

    @pl.loop(0, NSEG)
    def _(s):
        for cp in yb_copies(s):
            cp.wait()


@functools.partial(jax.jit, static_argnames=("B_seg_len",))
def pallas_concat_heads__spectral_gfnet__memory_aug_recurrent_mem_tr__prompt_kernel(
    A_x, A_w_r, A_w_i, B_x, B_mem0, B_Wq, B_Wk, B_Wv, B_Wo, B_seg_len,
):
    assert A_x.shape == (1, S, D) and B_x.shape == (1, S, D) and B_mem0.shape == (1, M, D)
    assert A_w_r.shape == (S, D // 2 + 1) and B_Wq.shape == (D, H, DH) and B_Wo.shape == (H, DH, D)
    assert B_seg_len == SEG
    hbm = pl.BlockSpec(memory_space=pl.ANY)
    out = pl.pallas_call(
        _kernel,
        out_shape=jax.ShapeDtypeStruct((S // 16, 16, 2 * D), bf16),
        in_specs=[hbm, hbm, hbm, hbm, pl.BlockSpec(memory_space=pltpu.VMEM), hbm, hbm, hbm, hbm],
        out_specs=hbm,
        scratch_shapes=[
            pltpu.VMEM((8, 128, D), i32),
            pltpu.VMEM((16, D // 4, 128), i32),
            pltpu.VMEM((16, D // 4, 128), i32),
            pltpu.VMEM((1, S), bf16),
            pltpu.VMEM((1, S), bf16),
            pltpu.VMEM((4, 256, 256), bf16),
            pltpu.VMEM((16, 256, 256), bf16),
            pltpu.VMEM((65, 16, 8, 256), f32),
            pltpu.VMEM((8, 128, D), i32),
            pltpu.VMEM((3, H // 2, D // 16, 2, 8, DH), i32),
            pltpu.VMEM((8, H * DH, 128), bf16),
            pltpu.VMEM((S, D), bf16),
            pltpu.VMEM((L, D), f32),
            pltpu.VMEM((S, D), bf16),
            pltpu.SemaphoreType.DMA((8,)),
            pltpu.SemaphoreType.DMA((1,)),
            pltpu.SemaphoreType.DMA((3 * H // 2,)),
            pltpu.SemaphoreType.DMA((1,)),
            pltpu.SemaphoreType.DMA((NXCHUNK,)),
            pltpu.SemaphoreType.DMA((1,)),
            pltpu.SemaphoreType.DMA((1,)),
        ],
        compiler_params=pltpu.CompilerParams(vmem_limit_bytes=100 * 1024 * 1024),
    )(
        A_x.reshape(S // 16, 16, D), A_w_r.T, A_w_i.T,
        B_x.reshape(S, D), B_mem0.reshape(M, D),
        B_Wq.reshape(D // 16, 8, 2, H, DH), B_Wk.reshape(D // 16, 8, 2, H, DH),
        B_Wv.reshape(D // 16, 8, 2, H, DH), B_Wo.reshape(H * DH, D),
    )
    return out.reshape(1, S, 2 * D)
```

```python
import functools
import math

import jax
import jax.numpy as jnp
from jax import lax
import jax.experimental.pallas as pl
import jax.experimental.pallas.tpu as pltpu

bf16, f32, i32 = jnp.bfloat16, jnp.float32, jnp.int32

S, D = 2048, 1024
H, DH = 32, 128
M, SEG = 8, 32
L = M + SEG
NSEG = S // SEG
XCHUNK = 128
NXCHUNK = S // XCHUNK
SCHUNK = XCHUNK // SEG

_NN = (((1,), (0,)), ((), ()))
_NT = (((1,), (1,)), ((), ()))
_HI16 = -65536
_R2 = math.sqrt(0.5)
_SCALE = 2.0 ** -5


def _dot(a, b, dims=_NN):
    return lax.dot_general(a, b, dims, preferred_element_type=f32)


def _lo_f32(w):
    return pltpu.bitcast(w << 16, f32)


def _hi_f32(w):
    return pltpu.bitcast(w & _HI16, f32)


def _cadd(a, b):
    return a[0] + b[0], a[1] + b[1]


def _csub(a, b):
    return a[0] - b[0], a[1] - b[1]


def _fft4(x0, x1, x2, x3, sign):
    a, b = _cadd(x0, x2), _csub(x0, x2)
    c, d = _cadd(x1, x3), _csub(x1, x3)
    minus_i = (b[0] + d[1], b[1] - d[0])
    plus_i = (b[0] - d[1], b[1] + d[0])
    if sign < 0:
        return _cadd(a, c), minus_i, _csub(a, c), plus_i
    return _cadd(a, c), plus_i, _csub(a, c), minus_i


def _twiddle16(x, m, sign):
    if m == 0:
        return x
    if m == 4:
        return (-x[1], x[0]) if sign > 0 else (x[1], -x[0])
    if m == 2:
        if sign > 0:
            return (x[0] - x[1]) * _R2, (x[0] + x[1]) * _R2
        return (x[0] + x[1]) * _R2, (x[1] - x[0]) * _R2
    if m == 6:
        if sign > 0:
            return (x[0] + x[1]) * -_R2, (x[0] - x[1]) * _R2
        return (x[1] - x[0]) * _R2, (x[0] + x[1]) * -_R2
    c, s = math.cos(2 * math.pi * m / 16), sign * math.sin(2 * math.pi * m / 16)
    return x[0] * c - x[1] * s, x[0] * s + x[1] * c


def _fft16(x, sign):
    t = [None] * 16
    for a0 in range(4):
        ys = _fft4(x[a0], x[4 + a0], x[8 + a0], x[12 + a0], sign)
        for k0 in range(4):
            t[4 * a0 + k0] = _twiddle16(ys[k0], a0 * k0, sign)
    y = [None] * 16
    for k0 in range(4):
        ys = _fft4(t[k0], t[4 + k0], t[8 + k0], t[12 + k0], sign)
        for k1 in range(4):
            y[k0 + 4 * k1] = ys[k1]
    return y


def _rfft8(x):
    s04, d04 = x[0] + x[4], x[0] - x[4]
    s26, d26 = x[2] + x[6], x[2] - x[6]
    s15, d15 = x[1] + x[5], x[1] - x[5]
    s37, d37 = x[3] + x[7], x[3] - x[7]
    e, o = s04 + s26, s15 + s37
    p, q = (d15 - d37) * _R2, (d15 + d37) * _R2
    return (e + o, e - o), (d04 + p, -(d26 + q)), (s04 - s26, s37 - s15), (d04 - p, d26 - q)


def _irfft8(r0, r1, r2, r3):
    a0, a4 = r0[0] + r0[1], r0[0] - r0[1]
    e0, e2 = a0 + r2[0], a0 - r2[0]
    e1, e3 = a4 - r2[1], a4 + r2[1]
    o0, o2 = r1[0] + r3[0], r3[1] - r1[1]
    dr, si = r1[0] - r3[0], r1[1] + r3[1]
    o1, o3 = (dr - si) * _R2, (dr + si) * -_R2
    return [e0 + o0, e1 + o1, e2 + o2, e3 + o3, e0 - o0, e1 - o1, e2 - o2, e3 - o3]


def _words(x):
    return pltpu.bitcast(x.astype(bf16), i32)


def _halves(w):
    return pltpu.bitcast(w, bf16)


def _matrix(m, i, rows=slice(0, 128)):
    return jnp.concatenate([_halves(m[i, 0, rows, :]), _halves(m[i, 1, rows, :])], axis=1)


def _build_dft_matrices(m1, m2):
    ri = lax.broadcasted_iota(i32, (128, 128), 0)
    ci = lax.broadcasted_iota(i32, (128, 128), 1)
    ang = ((ri * ci) & 127).astype(f32) * (2 * math.pi / 128)
    cb, sb = jnp.cos(ang), jnp.sin(ang)
    ang = (ri[0:16] * ci[0:16]).astype(f32) * (2 * math.pi / S)
    ct_all, st_all = jnp.cos(ang) * _SCALE, jnp.sin(ang) * _SCALE

    def rotated(rows, a):
        ct, st = ct_all[a:a + 1], st_all[a:a + 1]
        return cb[0:rows] * ct - sb[0:rows] * st, sb[0:rows] * ct + cb[0:rows] * st

    zero = jnp.zeros((64, 128), f32)
    for p in range(4):
        c0, s0 = rotated(64, 2 * p)
        c1, s1 = rotated(64, 2 * (4 if p == 0 else 8 - p))
        if p == 0:
            nyquist = jnp.where((ci[0:64] & 1) == 0, _SCALE, -_SCALE)
            blocks = [[c0, zero], [zero, c1],
                      [jnp.where(ri[0:64] == 0, nyquist, -s0), zero], [zero, -s1]]
        else:
            blocks = [[c0, s0], [c1, -s1], [-s0, c0], [-s1, -c1]]
        for i, pair in enumerate(blocks):
            for k in range(2):
                m1[p, k, i * 32:(i + 1) * 32, :] = _words(pair[k])
    for a in range(16):
        c, s = rotated(128, a)
        m2[a, 0, 0:64, :] = _words(c)
        m2[a, 1, 0:64, :] = _words(-s)
        m2[a, 0, 64:128, :] = _words(s)
        m2[a, 1, 64:128, :] = _words(c)


def _forward(xv, m1, m2, ubuf, gbuf, wait_x):
    sub = lax.broadcasted_iota(i32, (8, 128), 0)

    def butterflies(a, quarter):
        extract = (_lo_f32, _hi_f32)[a % 2]
        for g in range(2 * quarter, 2 * quarter + 2):
            u = _rfft8([extract(xv[a // 2, g * 16:(g + 1) * 16, j * 128:(j + 1) * 128])
                        for j in range(8)])
            for p in range(4):
                for k in range(2):
                    ubuf[a % 2, p, k, g * 8:(g + 1) * 8, :] = _words(u[p][k])

    def feature_stage(a, p):
        t = _dot(_matrix(m1, p), _matrix(ubuf.at[a % 2], p, slice(0, 64)), _NT)
        tr, ti = t[0:128], t[128:256]
        if p == 0:
            nyq = jnp.where(sub == 0, ti[0:8] * 0.5, 0.0)
            ti = jnp.concatenate([jnp.where(sub == 0, 0.0, ti[0:8]), ti[8:128],
                                  jnp.zeros((8, 128), f32)], axis=0)
            tr = jnp.concatenate([jnp.where(sub == 0, tr[0:8] * 0.5, tr[0:8]), tr[8:128], nyq],
                                 axis=0)
        return jnp.concatenate([tr, ti], axis=1)

    def sequence_stage(a, p, t):
        g = _dot(t, _matrix(m2, a))
        for blk in range(16):
            gbuf[p * 16 + blk, a] = g[blk * 8:(blk + 1) * 8]
        if p == 0:
            gbuf[64, a] = g[128:136]

    wait_x(0)
    for quarter in range(4):
        butterflies(0, quarter)
    pending = None
    for i in range(64):
        a, p = divmod(i, 4)
        if p == 0 and a % 2 == 1 and a < 15:
            wait_x((a + 1) // 2)
        t = feature_stage(a, p)
        if a < 15:
            butterflies(a + 1, p)
        if pending is not None:
            sequence_stage(*pending)
        pending = (a, p, t)
    sequence_stage(*pending)


def _filter_rows(g, gbuf, filt):
    xs = _fft16([(gbuf[g, a, :, 0:128], gbuf[g, a, :, 128:256]) for a in range(16)], -1)
    ys = []
    for k1 in range(16):
        wr, wi = filt(k1)
        xr, xi = xs[k1]
        ys.append((xr * wr - xi * wi, xr * wi + xi * wr))
    hs = _fft16(ys, +1)
    for a in range(16):
        gbuf[g, a, :, 0:128] = hs[a][0]
        gbuf[g, a, :, 128:256] = hs[a][1]


def _inverse(m1, m2, gbuf, rbuf, yv, between):
    lane = lax.broadcasted_iota(i32, (128, 128), 1)

    def sequence_stage(a, p):
        h = gbuf[p * 16:(p + 1) * 16, a].reshape(128, 256).astype(bf16)
        z = _dot(_matrix(m2, a), h, _NT)
        zr, zi = z[0:128], z[128:256]
        if p == 0:
            nyq = _dot(_matrix(m2, a, slice(0, 64)), gbuf[64, a].astype(bf16), _NT)
            zi = jnp.where(lane == 0, nyq[:, 0:1], zi)
        return jnp.concatenate([zr, zi], axis=1)

    def feature_stage(a, p, z):
        v = _dot(z, _matrix(m1, p))
        rbuf[a % 4, p, 0] = v[:, 0:128]
        rbuf[a % 4, p, 1] = v[:, 128:256]

    def butterflies(r, eighth):
        for g in range(2 * eighth, 2 * eighth + 2):
            rows = slice(g * 8, (g + 1) * 8)
            ys = [_irfft8(*[(rbuf[a % 4, p, 0, rows, :], rbuf[a % 4, p, 1, rows, :])
                            for p in range(4)]) for a in (2 * r, 2 * r + 1)]
            for j in range(8):
                even = pltpu.bitcast(ys[0][j].astype(bf16).astype(f32), i32)
                odd = pltpu.bitcast(ys[1][j].astype(bf16).astype(f32), i32)
                yv[r, rows, j * 128:(j + 1) * 128] = lax.shift_right_logical(even, 16) | odd

    pending = None
    for i in range(64 + 9):
        z = None
        if i < 64:
            between(i)
            z = sequence_stage(*divmod(i, 4))
        if pending is not None:
            feature_stage(*divmod(i - 1, 4), pending)
        pending = z
        if i >= 9:
            butterflies(*divmod(i - 9, 8))


def _interleave_heads(w, j):
    for c in range(0, D // 16, 4):
        even, odd = w[j, c:c + 4, 0], w[j, c:c + 4, 1]
        w[j, c:c + 4, 0] = (even & 0xFFFF) | (odd << 16)
        w[j, c:c + 4, 1] = lax.shift_right_logical(even, 16) | (odd & _HI16)


def _head_weight(w, j, e):
    return _halves(w[j, :, e].reshape(D // 2, DH))


def _segment(s, wqkv, wo32, xs, qz, h_ref, outs):
    r0 = pl.multiple_of(s * SEG, SEG)
    z0 = pl.multiple_of(s * 8, 8)
    h_ref[M:L, :] = xs[s].astype(f32)
    row = lax.broadcasted_iota(i32, (L, L), 0)
    col = lax.broadcasted_iota(i32, (L, L), 1)
    mask = (row < M) | (row >= col)

    def project(h):
        wq, wk, wv = [_head_weight(w, h // 2, h % 2) for w in wqkv]
        q = jnp.concatenate([_dot(h_ref[0:L - 8, :], wq), qz[h, pl.ds(z0, 8), :]], axis=0)
        return q, _dot(h_ref[...], wk), _dot(h_ref[...], wv)

    def probabilities(q, k):
        sc = _dot(q, k.astype(bf16), _NT) * DH ** -0.5
        sc = jnp.where(mask, sc, -1e9)
        e = jnp.exp(sc - jnp.max(sc, axis=-1, keepdims=True))
        return e * pltpu.reciprocal(jnp.sum(e, axis=-1, keepdims=True), approx=False)

    def out_proj(o, n, lo, hi):
        w = pltpu.bitcast(wo32[n, lo * DH // 2:hi * DH // 2, :], bf16)
        return _dot(jnp.concatenate(o[lo:hi], axis=1), w)

    lag_scores, lag_mix, split = 2, 4, 24
    state, o, part = {}, [None] * H, [None] * 8
    for t in range(H + 8):
        if t < H:
            state[t] = project(t)
        else:
            part[t - H] = out_proj(o, t - H, 0, split)
        if 0 <= t - lag_scores < H:
            q, k, v = state[t - lag_scores]
            state[t - lag_scores] = (probabilities(q, k), v)
        if 0 <= t - lag_mix < H:
            p, v = state.pop(t - lag_mix)
            o[t - lag_mix] = _dot(p, v.astype(bf16))
    for n in range(8):
        res = out_proj(o, n, split, H) + part[n]
        h_ref[0:M, n * 128:(n + 1) * 128] = res[0:M]
        outs[pl.ds(r0, SEG), n * 128:(n + 1) * 128] = res[M:L].astype(bf16)


def _kernel(ax_hbm, wr_hbm, wi_hbm, bx_hbm, mem0_ref, wq_hbm, wk_hbm, wv_hbm, wo_hbm, out_hbm,
            xv, wrv, wiv, wnr, wni, m1, m2, ubuf, gbuf, rbuf, yv,
            wq_ref, wk_ref, wv_ref, wo, xs, xz_raw, xz, qz, h_ref, outs,
            sem_ax, sem_f, sem_w, sem_wo, sem_bx, sem_xz, sem_ya, sem_yb):
    wqkv = (wq_ref, wk_ref, wv_ref)
    ax32 = ax_hbm.bitcast(i32)
    out32 = out_hbm.bitcast(i32)

    def ax_copy(r):
        return pltpu.make_async_copy(ax32.at[:, r, :], xv.at[r], sem_ax.at[r])

    def ya_copy(r):
        return pltpu.make_async_copy(yv.at[r], out32.at[:, r, pl.ds(0, D)], sem_ya.at[0])

    def w_copies(m, j):
        w32 = (wq_hbm, wk_hbm, wv_hbm)[m].bitcast(i32)
        return [pltpu.make_async_copy(w32.at[:, :, e, j, :], wqkv[m].at[j, :, e],
                                      sem_w.at[m * (H // 2) + j]) for e in range(2)]

    def bx_copy(c):
        return pltpu.make_async_copy(bx_hbm.at[pl.ds(c * SCHUNK, SCHUNK)],
                                     xs.at[pl.ds(c * SCHUNK, SCHUNK)], sem_bx.at[c])

    def yb_copies(s):
        return [pltpu.make_async_copy(outs.at[pl.ds(pl.multiple_of(s * SEG + 16 * i, 16), 16)],
                                      out_hbm.at[2 * s + i, :, pl.ds(D, D)], sem_yb.at[0])
                for i in range(SEG // 16)]

    f_copies = [pltpu.make_async_copy(src.at[pl.ds(0, D // 2), pl.ds(k1 * 128, 128)],
                                      dst.at[k1].bitcast(bf16), sem_f.at[0])
                for k1 in range(16) for src, dst in ((wr_hbm, wrv), (wi_hbm, wiv))]
    f_copies += [pltpu.make_async_copy(src.at[pl.ds(D // 2, 1), :], dst, sem_f.at[0])
                 for src, dst in ((wr_hbm, wnr), (wi_hbm, wni))]
    wo_copies = [pltpu.make_async_copy(wo_hbm.at[:, pl.ds(n * 128, 128)], wo.at[n], sem_wo.at[0])
                 for n in range(8)]

    def start_pair(m, j):
        for cp in w_copies(m, j):
            cp.start()

    def wait_pair(m, j):
        for cp in w_copies(m, j):
            cp.wait()

    for r in range(8):
        ax_copy(r).start()
    xz_copy = pltpu.make_async_copy(bx_hbm.at[:, pl.ds(SEG - 8, 8), :], xz_raw, sem_xz.at[0])
    xz_copy.start()
    for cp in f_copies:
        cp.start()

    _build_dft_matrices(m1, m2)

    def wait_x(r):
        for j in (2 * r, 2 * r + 1):
            start_pair(0, j)
        ax_copy(r).wait()

    _forward(xv, m1, m2, ubuf, gbuf, wait_x)
    for j in range(H // 2):
        start_pair(1, j)

    for cp in f_copies:
        cp.wait()

    @pl.loop(0, 32)
    def _(i):
        c, jg = i // 8, i % 8
        for e, extract in enumerate((_lo_f32, _hi_f32)):
            k1 = 2 * c + e
            g = jnp.where(k1 < 4, 16 * k1, 16 * ((8 - k1) % 4) + 8) + jg
            _filter_rows(g, gbuf, lambda k: tuple(
                extract(w[k, pl.ds(32 * jg + c, 8, stride=4), :]) for w in (wrv, wiv)))

    _filter_rows(64, gbuf, lambda k: tuple(
        jnp.broadcast_to(w[:, k * 128:(k + 1) * 128].astype(f32), (8, 128)) for w in (wnr, wni)))

    def start_wv(i):
        if i % 32 == 0:
            for j in range(8):
                start_pair(2, i // 4 + j)

    _inverse(m1, m2, gbuf, rbuf, yv, start_wv)
    bx_copy(0).start()
    for cp in wo_copies:
        cp.start()

    xz_copy.wait()
    xz[...] = xz_raw[...].astype(f32).reshape(NSEG * 8, D).astype(bf16)
    for j in range(H // 2):
        wait_pair(0, j)
    _interleave_heads(wq_ref, 0)

    def early_queries(j, first=False, last=False):
        wait_pair(1, j)
        if not first:
            wait_pair(2, j - 1)
        _interleave_heads(wk_ref, j)
        if not first:
            _interleave_heads(wv_ref, j - 1)
        for e in range(2):
            wq = _head_weight(wq_ref, j, e)
            for i in range(4):
                rows = slice(i * 128, (i + 1) * 128)
                qz[2 * j + e, rows, :] = _dot(xz[rows, :], wq)
        if not last:
            _interleave_heads(wq_ref, j + 1)

    early_queries(0, first=True)

    @pl.loop(1, H // 2 - 1, unroll=2)
    def _(j):
        early_queries(j)

    early_queries(H // 2 - 1, last=True)
    wait_pair(2, H // 2 - 1)
    _interleave_heads(wv_ref, H // 2 - 1)

    for cp in wo_copies:
        cp.wait()
    for c in range(1, NXCHUNK):
        bx_copy(c).start()
    for r in range(8):
        ya_copy(r).start()
    h_ref[0:M, :] = mem0_ref[...].astype(f32)
    wo32 = wo.bitcast(i32)

    @pl.loop(0, NXCHUNK)
    def _(c):
        bx_copy(c).wait()

        @pl.loop(0, XCHUNK // SEG)
        def _(i):
            s = c * (XCHUNK // SEG) + i
            _segment(s, wqkv, wo32, xs, qz, h_ref, outs)
            for cp in yb_copies(s):
                cp.start()

    for r in range(8):
        ya_copy(r).wait()

    @pl.loop(0, NSEG)
    def _(s):
        for cp in yb_copies(s):
            cp.wait()


@functools.partial(jax.jit, static_argnames=("B_seg_len",))
def pallas_concat_heads__spectral_gfnet__memory_aug_recurrent_mem_tr__prompt_kernel(
    A_x, A_w_r, A_w_i, B_x, B_mem0, B_Wq, B_Wk, B_Wv, B_Wo, B_seg_len,
):
    assert A_x.shape == (1, S, D) and B_x.shape == (1, S, D) and B_mem0.shape == (1, M, D)
    assert A_w_r.shape == (S, D // 2 + 1) and B_Wq.shape == (D, H, DH) and B_Wo.shape == (H, DH, D)
    assert B_seg_len == SEG
    hbm = pl.BlockSpec(memory_space=pl.ANY)
    out = pl.pallas_call(
        _kernel,
        out_shape=jax.ShapeDtypeStruct((S // 16, 16, 2 * D), bf16),
        in_specs=[hbm, hbm, hbm, hbm, pl.BlockSpec(memory_space=pltpu.VMEM), hbm, hbm, hbm, hbm],
        out_specs=hbm,
        scratch_shapes=[
            pltpu.VMEM((8, 128, D), i32),
            pltpu.VMEM((16, D // 4, 128), i32),
            pltpu.VMEM((16, D // 4, 128), i32),
            pltpu.VMEM((1, S), bf16),
            pltpu.VMEM((1, S), bf16),
            pltpu.VMEM((4, 2, 128, 128), i32),
            pltpu.VMEM((16, 2, 128, 128), i32),
            pltpu.VMEM((2, 4, 2, 64, 128), i32),
            pltpu.VMEM((65, 16, 8, 256), f32),
            pltpu.VMEM((4, 4, 2, 128, 128), f32),
            pltpu.VMEM((8, 128, D), i32),
            pltpu.VMEM((H // 2, D // 16, 2, 8, DH), i32),
            pltpu.VMEM((H // 2, D // 16, 2, 8, DH), i32),
            pltpu.VMEM((H // 2, D // 16, 2, 8, DH), i32),
            pltpu.VMEM((8, H * DH, 128), bf16),
            pltpu.VMEM((NSEG, SEG, D), bf16),
            pltpu.VMEM((NSEG, 8, D), bf16),
            pltpu.VMEM((NSEG * 8, D), bf16),
            pltpu.VMEM((H, NSEG * 8, DH), f32),
            pltpu.VMEM((L, D), f32),
            pltpu.VMEM((S, D), bf16),
            pltpu.SemaphoreType.DMA((8,)),
            pltpu.SemaphoreType.DMA((1,)),
            pltpu.SemaphoreType.DMA((3 * H // 2,)),
            pltpu.SemaphoreType.DMA((1,)),
            pltpu.SemaphoreType.DMA((NXCHUNK,)),
            pltpu.SemaphoreType.DMA((1,)),
            pltpu.SemaphoreType.DMA((1,)),
            pltpu.SemaphoreType.DMA((1,)),
        ],
        compiler_params=pltpu.CompilerParams(vmem_limit_bytes=100 * 1024 * 1024),
    )(
        A_x.reshape(S // 16, 16, D), A_w_r.T, A_w_i.T,
        B_x.reshape(NSEG, SEG, D), B_mem0.reshape(M, D),
        B_Wq.reshape(D // 16, 8, 2, H, DH), B_Wk.reshape(D // 16, 8, 2, H, DH),
        B_Wv.reshape(D // 16, 8, 2, H, DH), B_Wo.reshape(H * DH, D),
    )
    return out.reshape(1, S, 2 * D)
```

```python
import functools
import math

import jax
import jax.numpy as jnp
from jax import lax
import jax.experimental.pallas as pl
import jax.experimental.pallas.tpu as pltpu

bf16, f32, i32 = jnp.bfloat16, jnp.float32, jnp.int32

S, D = 2048, 1024
H, DH = 32, 128
M, SEG = 8, 32
L = M + SEG
NSEG = S // SEG
NBUILD = 8
NPAIR = H // 2
EARLY_ITEMS = 22
XCHUNK = 64
NXCHUNK = S // XCHUNK
SCHUNK = XCHUNK // SEG

_NN = (((1,), (0,)), ((), ()))
_NT = (((1,), (1,)), ((), ()))
_HI16 = -65536
_R2 = math.sqrt(0.5)
_SCALE = 2.0 ** -5


def _dot(a, b, dims=_NN):
    return lax.dot_general(a, b, dims, preferred_element_type=f32)


def _lo_f32(w):
    return pltpu.bitcast(w << 16, f32)


def _hi_f32(w):
    return pltpu.bitcast(w & _HI16, f32)


def _cadd(a, b):
    return a[0] + b[0], a[1] + b[1]


def _csub(a, b):
    return a[0] - b[0], a[1] - b[1]


def _fft4(x0, x1, x2, x3, sign):
    a, b = _cadd(x0, x2), _csub(x0, x2)
    c, d = _cadd(x1, x3), _csub(x1, x3)
    minus_i = (b[0] + d[1], b[1] - d[0])
    plus_i = (b[0] - d[1], b[1] + d[0])
    if sign < 0:
        return _cadd(a, c), minus_i, _csub(a, c), plus_i
    return _cadd(a, c), plus_i, _csub(a, c), minus_i


def _twiddle16(x, m, sign):
    if m == 0:
        return x
    if m == 4:
        return (-x[1], x[0]) if sign > 0 else (x[1], -x[0])
    if m == 2:
        if sign > 0:
            return (x[0] - x[1]) * _R2, (x[0] + x[1]) * _R2
        return (x[0] + x[1]) * _R2, (x[1] - x[0]) * _R2
    if m == 6:
        if sign > 0:
            return (x[0] + x[1]) * -_R2, (x[0] - x[1]) * _R2
        return (x[1] - x[0]) * _R2, (x[0] + x[1]) * -_R2
    c, s = math.cos(2 * math.pi * m / 16), sign * math.sin(2 * math.pi * m / 16)
    return x[0] * c - x[1] * s, x[0] * s + x[1] * c


def _rfft8(x):
    s04, d04 = x[0] + x[4], x[0] - x[4]
    s26, d26 = x[2] + x[6], x[2] - x[6]
    s15, d15 = x[1] + x[5], x[1] - x[5]
    s37, d37 = x[3] + x[7], x[3] - x[7]
    e, o = s04 + s26, s15 + s37
    p, q = (d15 - d37) * _R2, (d15 + d37) * _R2
    return (e + o, e - o), (d04 + p, -(d26 + q)), (s04 - s26, s37 - s15), (d04 - p, d26 - q)


def _irfft8(r0, r1, r2, r3):
    a0, a4 = r0[0] + r0[1], r0[0] - r0[1]
    e0, e2 = a0 + r2[0], a0 - r2[0]
    e1, e3 = a4 - r2[1], a4 + r2[1]
    o0, o2 = r1[0] + r3[0], r3[1] - r1[1]
    dr, si = r1[0] - r3[0], r1[1] + r3[1]
    o1, o3 = (dr - si) * _R2, (dr + si) * -_R2
    return [e0 + o0, e1 + o1, e2 + o2, e3 + o3, e0 - o0, e1 - o1, e2 - o2, e3 - o3]


def _words(x):
    return pltpu.bitcast(x.astype(bf16), i32)


def _halves(w):
    return pltpu.bitcast(w, bf16)


def _matrix(m, i, rows=slice(0, 128)):
    return jnp.concatenate([_halves(m[i, 0, rows, :]), _halves(m[i, 1, rows, :])], axis=1)


def _build_dft_matrices(m1, m2):
    ri = lax.broadcasted_iota(i32, (128, 128), 0)
    ci = lax.broadcasted_iota(i32, (128, 128), 1)
    ang = ((ri * ci) & 127).astype(f32) * (2 * math.pi / 128)
    cb, sb = jnp.cos(ang), jnp.sin(ang)
    ang = (ri[0:16] * ci[0:16]).astype(f32) * (2 * math.pi / S)
    ct_all, st_all = jnp.cos(ang) * _SCALE, jnp.sin(ang) * _SCALE

    def rotated(rows, a):
        ct, st = ct_all[a:a + 1], st_all[a:a + 1]
        return cb[0:rows] * ct - sb[0:rows] * st, sb[0:rows] * ct + cb[0:rows] * st

    for p in range(4):
        c0, s0 = rotated(64, 2 * p)
        c1, s1 = rotated(64, 2 * (4 if p == 0 else 8 - p))
        if p == 0:
            nyquist = jnp.where((ci[0:64] & 1) == 0, _SCALE, -_SCALE)
            blocks = [[c0, c1], [jnp.where(ri[0:64] == 0, nyquist, -s0), -s1]]
        else:
            blocks = [[c0, s0], [c1, -s1], [-s0, c0], [-s1, -c1]]
        for i, pair in enumerate(blocks):
            for k in range(2):
                m1[p, k, i * 32:(i + 1) * 32, :] = _words(pair[k])

    def build_m2(a):
        c, s = rotated(128, a)
        m2[a, 0, 0:64, :] = _words(c)
        m2[a, 1, 0:64, :] = _words(-s)
        m2[a, 0, 64:128, :] = _words(s)
        m2[a, 1, 64:128, :] = _words(c)

    return build_m2


def _forward(xv, m1, m2, ubuf, gbuf, wait_x, build_m2):
    sub = lax.broadcasted_iota(i32, (8, 128), 0)

    def butterflies(a, quarter):
        extract = (_lo_f32, _hi_f32)[a % 2]
        for g in range(2 * quarter, 2 * quarter + 2):
            u = _rfft8([extract(xv[a // 2, g * 16:(g + 1) * 16, j * 128:(j + 1) * 128])
                        for j in range(8)])
            for p in range(4):
                for k in range(2):
                    ubuf[a % 2, p, k, g * 8:(g + 1) * 8, :] = _words(u[p][k])

    def feature_stage(a, p):
        if p > 0:
            t = _dot(_matrix(m1, p), _matrix(ubuf.at[a % 2], p, slice(0, 64)), _NT)
            return jnp.concatenate([t[0:128], t[128:256]], axis=1)
        t0, t1 = [_dot(_halves(m1[0, k, 0:64, :]), _halves(ubuf[a % 2, 0, k]), _NT)
                  for k in range(2)]
        tr = [jnp.where(sub == 0, t0[0:8] * 0.5, t0[0:8]), t0[8:64], t1[0:64],
              jnp.where(sub == 0, t0[64:72] * 0.5, 0.0)]
        ti = [jnp.where(sub == 0, 0.0, t0[64:72]), t0[72:128], t1[64:128],
              jnp.zeros((8, 128), f32)]
        return jnp.concatenate([jnp.concatenate(tr, axis=0), jnp.concatenate(ti, axis=0)], axis=1)

    def sequence_stage(a, p, t):
        g = _dot(t, _matrix(m2, a))
        for blk in range(16):
            gbuf[p * 16 + blk, a] = g[blk * 8:(blk + 1) * 8]
        if p == 0:
            gbuf[64, a] = g[128:136]

    for a in range(NBUILD):
        build_m2(a)
    wait_x(0)
    for quarter in range(4):
        butterflies(0, quarter)
    pending = None
    for i in range(64):
        a, p = divmod(i, 4)
        if p == 0 and a % 2 == 1 and a < 15:
            wait_x((a + 1) // 2)
        t = feature_stage(a, p)
        if a < 15:
            butterflies(a + 1, p)
        if p == 1 and a + NBUILD < 16:
            build_m2(a + NBUILD)
        if pending is not None:
            sequence_stage(*pending)
        pending = (a, p, t)
    sequence_stage(*pending)


def _filter_rows(g, gbuf, filt):
    def load(slots):
        return [(gbuf[g, a, :, 0:128], gbuf[g, a, :, 128:256]) for a in slots]

    def store(slots, values):
        for a, (re, im) in zip(slots, values):
            gbuf[g, a, :, 0:128] = re
            gbuf[g, a, :, 128:256] = im

    for a0 in range(4):
        slots = range(a0, 16, 4)
        ys = _fft4(*load(slots), -1)
        store(slots, [_twiddle16(ys[k0], a0 * k0, -1) for k0 in range(4)])
        yield
    for k0 in range(4):
        slots = range(4 * k0, 4 * k0 + 4)
        ys = []
        for k1, (xr, xi) in enumerate(_fft4(*load(slots), -1)):
            wr, wi = filt(k0 + 4 * k1)
            ys.append((xr * wr - xi * wi, xr * wi + xi * wr))
        ys = _fft4(*ys, +1)
        store(slots, [_twiddle16(ys[a0], a0 * k0, +1) for a0 in range(4)])
        yield
    for a0 in range(4):
        slots = range(a0, 16, 4)
        store(slots, _fft4(*load(slots), +1))
        yield


def _inverse(m1, m2, gbuf, rbuf, yv):
    def sequence_stage(a, p):
        h = gbuf[p * 16:(p + 1) * 16, a].reshape(128, 256)
        if p > 0:
            z = _dot(_matrix(m2, a), h.astype(bf16), _NT)
            return [jnp.concatenate([z[0:128], z[128:256]], axis=1)]
        sub = lax.broadcasted_iota(i32, (8, 256), 0)
        turned = jnp.concatenate([h[:, 128:256], -h[:, 0:128]], axis=1)
        low = [h[0:64], jnp.where(sub == 0, gbuf[64, a], turned[0:8]), turned[8:64]]
        high = [h[64:128], turned[64:128]]
        return [_dot(_matrix(m2, a, slice(0, 64)), jnp.concatenate(rows, axis=0).astype(bf16), _NT)
                for rows in (low, high)]

    def feature_stage(a, p, z):
        if p > 0:
            v = _dot(z[0], _matrix(m1, p))
            v = (v[:, 0:128], v[:, 128:256])
        else:
            v = [_dot(z[k], _halves(m1[0, k, 0:64, :])) for k in range(2)]
        rbuf[a % 4, p, 0] = v[0]
        rbuf[a % 4, p, 1] = v[1]

    def butterflies(r, eighth):
        for g in range(2 * eighth, 2 * eighth + 2):
            rows = slice(g * 8, (g + 1) * 8)
            ys = [_irfft8(*[(rbuf[a % 4, p, 0, rows, :], rbuf[a % 4, p, 1, rows, :])
                            for p in range(4)]) for a in (2 * r, 2 * r + 1)]
            for j in range(8):
                even = pltpu.bitcast(ys[0][j].astype(bf16).astype(f32), i32)
                odd = pltpu.bitcast(ys[1][j].astype(bf16).astype(f32), i32)
                yv[r, rows, j * 128:(j + 1) * 128] = lax.shift_right_logical(even, 16) | odd

    pending = None
    for i in range(64 + 9):
        z = None
        if i < 64:
            z = sequence_stage(*divmod(i, 4))
        if pending is not None:
            feature_stage(*divmod(i - 1, 4), pending)
        pending = z
        if i >= 9:
            butterflies(*divmod(i - 9, 8))


def _interleave_heads(w, items, pieces=1):
    per_piece = D // 16 // pieces
    for first in range(0, D // 16, per_piece):
        for i in items:
            for c in range(first, first + per_piece, 2):
                even, odd = w[i, c:c + 2, 0], w[i, c:c + 2, 1]
                w[i, c:c + 2, 0] = (even & 0xFFFF) | (odd << 16)
                w[i, c:c + 2, 1] = lax.shift_right_logical(even, 16) | (odd & _HI16)
        yield


def _head_weight(w, i, e):
    return _halves(w[i, :, e].reshape(D // 2, DH))


def _segment(s, wqkv, wo32, xs, early_rows, h_ref, outs):
    z0 = pl.multiple_of(s * 8, 8)
    h_ref[M:L, :] = xs[s].astype(f32)
    row = lax.broadcasted_iota(i32, (L, L), 0)
    col = lax.broadcasted_iota(i32, (L, L), 1)
    mask = (row < M) | (row >= col)

    def project(h):
        items = [m * NPAIR + h // 2 for m in range(3)]
        ws = [_head_weight(wqkv, i, h % 2) for i in items]
        rows = [L - 8 if i < EARLY_ITEMS else L for i in items]
        if h == 0:
            first = [_dot(h_ref[0:n, 0:D // 2], w[0:D // 2]) for n, w in zip(rows, ws)]
            qkv = [_dot(h_ref[0:n, D // 2:D], w[D // 2:D]) + f for n, w, f in zip(rows, ws, first)]
        else:
            qkv = [_dot(h_ref[0:n, :], w) for n, w in zip(rows, ws)]
        return [jnp.concatenate([v, early_rows[2 * i + h % 2, pl.ds(z0, 8), :]], axis=0)
                if i < EARLY_ITEMS else v for v, i in zip(qkv, items)]

    def probabilities(q, k):
        sc = _dot(q, k.astype(bf16), _NT) * DH ** -0.5
        sc = jnp.where(mask, sc, -1e9)
        e = jnp.exp(sc - jnp.max(sc, axis=-1, keepdims=True))
        return e * pltpu.reciprocal(jnp.sum(e, axis=-1, keepdims=True), approx=False)

    def out_proj(o, n, lo, hi):
        w = pltpu.bitcast(wo32[n, lo * DH // 2:hi * DH // 2, :], bf16)
        return _dot(jnp.concatenate(o[lo:hi], axis=1), w)

    lag_scores, lag_mix, split = 2, 4, 24
    state, o, part = {}, [None] * H, [None] * 8
    for t in range(H + 8):
        if t < H:
            state[t] = project(t)
        else:
            part[t - H] = out_proj(o, t - H, 0, split)
        if 0 <= t - lag_scores < H:
            q, k, v = state[t - lag_scores]
            state[t - lag_scores] = (probabilities(q, k), v)
        if 0 <= t - lag_mix < H:
            p, v = state.pop(t - lag_mix)
            o[t - lag_mix] = _dot(p, v.astype(bf16))
    for n in range(8):
        res = out_proj(o, n, split, H) + part[n]
        h_ref[0:M, n * 128:(n + 1) * 128] = res[0:M]
        for i in range(SEG // 16):
            outs[2 * s + i, :, n * 128:(n + 1) * 128] = res[M + 16 * i:M + 16 * i + 16].astype(bf16)


def _kernel(ax_hbm, wr_hbm, wi_hbm, bx_hbm, mem0_ref, wq_hbm, wk_hbm, wv_hbm, wo_hbm, out_hbm,
            xv, wrv, wiv, wnr, wni, m1, m2, ubuf, gbuf, rbuf, yv,
            wqkv, wo, xs, xz_raw, xz, early_rows, h_ref, outs,
            sem_ax, sem_f, sem_w, sem_wo, sem_bx, sem_xz, sem_ya, sem_yb):
    ax32 = ax_hbm.bitcast(i32)
    out32 = out_hbm.bitcast(i32)

    def ax_copy(r):
        return pltpu.make_async_copy(ax32.at[:, r, :], xv.at[r], sem_ax.at[r])

    def ya_copy(r):
        return pltpu.make_async_copy(yv.at[r], out32.at[:, r, pl.ds(0, D)], sem_ya.at[0])

    def bx_copy(c):
        return pltpu.make_async_copy(bx_hbm.at[pl.ds(c * SCHUNK, SCHUNK)],
                                     xs.at[pl.ds(c * SCHUNK, SCHUNK)], sem_bx.at[c])

    def yb_copy(c):
        rows = pl.ds(c * (XCHUNK // 16), XCHUNK // 16)
        return pltpu.make_async_copy(outs.at[rows], out_hbm.at[rows, :, pl.ds(D, D)], sem_yb.at[0])

    f_copies = [pltpu.make_async_copy(src.at[pl.ds(0, D // 2), pl.ds(k1 * 128, 128)],
                                      dst.at[k1].bitcast(bf16), sem_f.at[0])
                for k1 in range(16) for src, dst in ((wr_hbm, wrv), (wi_hbm, wiv))]
    f_copies += [pltpu.make_async_copy(src.at[pl.ds(D // 2, 1), :], dst, sem_f.at[0])
                 for src, dst in ((wr_hbm, wnr), (wi_hbm, wni))]
    wo_copies = [pltpu.make_async_copy(wo_hbm.at[:, pl.ds(n * 128, 128)], wo.at[n], sem_wo.at[0])
                 for n in range(8)]

    def start_pair(m, j):
        w32 = (wq_hbm, wk_hbm, wv_hbm)[m].bitcast(i32)
        for e in range(2):
            pltpu.make_async_copy(w32.at[:, :, e, j, :], wqkv.at[m * NPAIR + j, :, e],
                                  sem_w.at[m * NPAIR + j]).start()

    def wait_item(i):
        pltpu.make_async_copy(wqkv.at[i], wqkv.at[i], sem_w.at[i]).wait()

    for r in range(8):
        ax_copy(r).start()
    xz_copy = pltpu.make_async_copy(bx_hbm.at[:, pl.ds(SEG - 8, 8), :], xz_raw, sem_xz.at[0])
    xz_copy.start()
    for j in range(4):
        start_pair(0, j)
    for cp in f_copies:
        cp.start()

    build_m2 = _build_dft_matrices(m1, m2)

    def wait_x(r):
        for j in {3: range(4, 10), 6: range(10, 16)}.get(r, ()):
            start_pair(0, j)
        for i in {0: (0,), 1: (1, 2), 3: (3, 4, 5), 6: (6, 7)}.get(r, ()):
            ax_copy(i).wait()

    _forward(xv, m1, m2, ubuf, gbuf, wait_x, build_m2)

    xz_copy.wait()
    xz[...] = xz_raw[...].astype(f32).reshape(NSEG * 8, D)

    def filter_groups(i):
        c, jg = i // 8, i % 8
        for e, extract in enumerate((_lo_f32, _hi_f32)):
            k1 = 2 * c + e
            g = jnp.where(k1 < 4, 16 * k1, 16 * ((8 - k1) % 4) + 8) + jg
            yield from _filter_rows(g, gbuf, lambda k: tuple(
                extract(w[k, pl.ds(32 * jg + c, 8, stride=4), :]) for w in (wrv, wiv)))

    def project_early(items, filter_work, interleave_work):
        for i in items:
            for e in range(2):
                for r0 in range(0, NSEG * 8, 64):
                    for _ in range(3):
                        next(filter_work, None)
                    res = _dot(xz[r0:r0 + 64, :], _head_weight(wqkv, i, e))
                    early_rows[2 * i + e, r0:r0 + 64, :] = res
                    gbuf[65 + i % 2, 0, :, 0:128] = res[0:8]
                    next(interleave_work, None)

    for i in range(2):
        wait_item(i)
    list(_interleave_heads(wqkv, (0, 1)))

    @pl.loop(0, 2)
    def _(i):
        wait_item(i + 2)
        project_early((i,), iter(()), _interleave_heads(wqkv, (i + 2,), 16))

    for cp in f_copies:
        cp.wait()

    @pl.loop(0, 8)
    def _(t):
        for m in (1, 2):
            @pl.when(t // 4 == m - 1)
            def _():
                for i in range(4):
                    start_pair(m, 4 * (t % 4) + i)

        ahead = (2 * t + 4, 2 * t + 5)
        for i in ahead:
            wait_item(i)
        filter_work = (x for i in range(4) for x in filter_groups(4 * t + i))
        project_early((2 * t + 2, 2 * t + 3), filter_work, _interleave_heads(wqkv, ahead, 32))

    bx_copy(0).start()
    for cp in wo_copies:
        cp.start()
    list(_filter_rows(64, gbuf, lambda k: tuple(
        jnp.broadcast_to(w[:, k * 128:(k + 1) * 128].astype(f32), (8, 128)) for w in (wnr, wni))))

    _inverse(m1, m2, gbuf, rbuf, yv)

    steps = EARLY_ITEMS - 18
    per_step = (3 * NPAIR - 20) // steps
    for i in range(20, 3 * NPAIR):
        wait_item(i)

    @pl.loop(0, steps)
    def _(t):
        ahead = [20 + per_step * t + i for i in range(per_step)]
        project_early((18 + t,), iter(()), _interleave_heads(wqkv, ahead, 16))

    list(_interleave_heads(wqkv, range(20 + per_step * steps, 3 * NPAIR)))

    for cp in wo_copies:
        cp.wait()
    for c in range(1, NXCHUNK):
        bx_copy(c).start()
    for r in range(8):
        ya_copy(r).start()
    h_ref[0:M, :] = mem0_ref[...].astype(f32)
    wo32 = wo.bitcast(i32)

    @pl.loop(0, NXCHUNK)
    def _(c):
        bx_copy(c).wait()

        for i in range(SCHUNK):
            _segment(c * SCHUNK + i, wqkv, wo32, xs, early_rows, h_ref, outs)
        yb_copy(c).start()

    for r in range(8):
        ya_copy(r).wait()
    for c in range(NXCHUNK):
        yb_copy(c).wait()


@functools.partial(jax.jit, static_argnames=("B_seg_len",))
def pallas_concat_heads__spectral_gfnet__memory_aug_recurrent_mem_tr__prompt_kernel(
    A_x, A_w_r, A_w_i, B_x, B_mem0, B_Wq, B_Wk, B_Wv, B_Wo, B_seg_len,
):
    assert A_x.shape == (1, S, D) and B_x.shape == (1, S, D) and B_mem0.shape == (1, M, D)
    assert A_w_r.shape == (S, D // 2 + 1) and B_Wq.shape == (D, H, DH) and B_Wo.shape == (H, DH, D)
    assert B_seg_len == SEG
    hbm = pl.BlockSpec(memory_space=pl.ANY)
    out = pl.pallas_call(
        _kernel,
        out_shape=jax.ShapeDtypeStruct((S // 16, 16, 2 * D), bf16),
        in_specs=[hbm, hbm, hbm, hbm, pl.BlockSpec(memory_space=pltpu.VMEM), hbm, hbm, hbm, hbm],
        out_specs=hbm,
        scratch_shapes=[
            pltpu.VMEM((8, 128, D), i32),
            pltpu.VMEM((16, D // 4, 128), i32),
            pltpu.VMEM((16, D // 4, 128), i32),
            pltpu.VMEM((1, S), bf16),
            pltpu.VMEM((1, S), bf16),
            pltpu.VMEM((4, 2, 128, 128), i32),
            pltpu.VMEM((16, 2, 128, 128), i32),
            pltpu.VMEM((2, 4, 2, 64, 128), i32),
            pltpu.VMEM((67, 16, 8, 256), f32),
            pltpu.VMEM((4, 4, 2, 128, 128), f32),
            pltpu.VMEM((8, 128, D), i32),
            pltpu.VMEM((3 * NPAIR, D // 16, 2, 8, DH), i32),
            pltpu.VMEM((8, H * DH, 128), bf16),
            pltpu.VMEM((NSEG, SEG, D), bf16),
            pltpu.VMEM((NSEG, 8, D), bf16),
            pltpu.VMEM((NSEG * 8, D), f32),
            pltpu.VMEM((2 * EARLY_ITEMS, NSEG * 8, DH), f32),
            pltpu.VMEM((L, D), f32),
            pltpu.VMEM((S // 16, 16, D), bf16),
            pltpu.SemaphoreType.DMA((8,)),
            pltpu.SemaphoreType.DMA((1,)),
            pltpu.SemaphoreType.DMA((3 * NPAIR,)),
            pltpu.SemaphoreType.DMA((1,)),
            pltpu.SemaphoreType.DMA((NXCHUNK,)),
            pltpu.SemaphoreType.DMA((1,)),
            pltpu.SemaphoreType.DMA((1,)),
            pltpu.SemaphoreType.DMA((1,)),
        ],
        compiler_params=pltpu.CompilerParams(vmem_limit_bytes=100 * 1024 * 1024),
    )(
        A_x.reshape(S // 16, 16, D), A_w_r.T, A_w_i.T,
        B_x.reshape(NSEG, SEG, D), B_mem0.reshape(M, D),
        B_Wq.reshape(D // 16, 8, 2, H, DH), B_Wk.reshape(D // 16, 8, 2, H, DH),
        B_Wv.reshape(D // 16, 8, 2, H, DH), B_Wo.reshape(H * DH, D),
    )
    return out.reshape(1, S, 2 * D)
```

```python
import functools
import math

import jax
import jax.numpy as jnp
from jax import lax
import jax.experimental.pallas as pl
import jax.experimental.pallas.tpu as pltpu

bf16, f32, i32 = jnp.bfloat16, jnp.float32, jnp.int32

S, D = 2048, 1024
H, DH = 32, 128
M, SEG = 8, 32
L = M + SEG
NSEG = S // SEG
NPAIR = H // 2
FIRST_ITEMS = 5
EARLY_ITEMS = 25
SCHUNK = 2
NCHUNK = NSEG // SCHUNK

_NN = (((1,), (0,)), ((), ()))
_NT = (((1,), (1,)), ((), ()))
_HI16 = -65536
_R2 = math.sqrt(0.5)
_SCALE = 2.0 ** -5


def _dot(a, b, dims=_NN):
    return lax.dot_general(a, b, dims, preferred_element_type=f32)


def _lo_f32(w):
    return pltpu.bitcast(w << 16, f32)


def _hi_f32(w):
    return pltpu.bitcast(w & _HI16, f32)


def _cadd(a, b):
    return a[0] + b[0], a[1] + b[1]


def _csub(a, b):
    return a[0] - b[0], a[1] - b[1]


def _fft4(x0, x1, x2, x3, sign):
    a, b = _cadd(x0, x2), _csub(x0, x2)
    c, d = _cadd(x1, x3), _csub(x1, x3)
    minus_i = (b[0] + d[1], b[1] - d[0])
    plus_i = (b[0] - d[1], b[1] + d[0])
    if sign < 0:
        return _cadd(a, c), minus_i, _csub(a, c), plus_i
    return _cadd(a, c), plus_i, _csub(a, c), minus_i


def _twiddle16(x, m, sign):
    if m == 0:
        return x
    if m == 4:
        return (-x[1], x[0]) if sign > 0 else (x[1], -x[0])
    if m == 2:
        if sign > 0:
            return (x[0] - x[1]) * _R2, (x[0] + x[1]) * _R2
        return (x[0] + x[1]) * _R2, (x[1] - x[0]) * _R2
    if m == 6:
        if sign > 0:
            return (x[0] + x[1]) * -_R2, (x[0] - x[1]) * _R2
        return (x[1] - x[0]) * _R2, (x[0] + x[1]) * -_R2
    c, s = math.cos(2 * math.pi * m / 16), sign * math.sin(2 * math.pi * m / 16)
    return x[0] * c - x[1] * s, x[0] * s + x[1] * c


def _rfft8(x):
    s04, d04 = x[0] + x[4], x[0] - x[4]
    s26, d26 = x[2] + x[6], x[2] - x[6]
    s15, d15 = x[1] + x[5], x[1] - x[5]
    s37, d37 = x[3] + x[7], x[3] - x[7]
    e, o = s04 + s26, s15 + s37
    p, q = (d15 - d37) * _R2, (d15 + d37) * _R2
    return (e + o, e - o), (d04 + p, -(d26 + q)), (s04 - s26, s37 - s15), (d04 - p, d26 - q)


def _irfft8(r0, r1, r2, r3):
    a0, a4 = r0[0] + r0[1], r0[0] - r0[1]
    e0, e2 = a0 + r2[0], a0 - r2[0]
    e1, e3 = a4 - r2[1], a4 + r2[1]
    o0, o2 = r1[0] + r3[0], r3[1] - r1[1]
    dr, si = r1[0] - r3[0], r1[1] + r3[1]
    o1, o3 = (dr - si) * _R2, (dr + si) * -_R2
    return [e0 + o0, e1 + o1, e2 + o2, e3 + o3, e0 - o0, e1 - o1, e2 - o2, e3 - o3]


def _halves(w):
    return pltpu.bitcast(w, bf16)


def _complex_product(apply, m, xr, xi, xs, conjugate):
    shared = apply(_halves(m[0]), xs)
    for_re, for_im = (2, 1) if conjugate else (1, 2)
    return apply(_halves(m[for_re]), xi) + shared, apply(_halves(m[for_im]), xr) + shared


def _from_left(m, x):
    return _dot(m, x, _NT)


def _from_right(m, x):
    return _dot(x, m)


def _build_dft_matrices(m1, m2):
    ri = lax.broadcasted_iota(i32, (128, 128), 0)
    ci = lax.broadcasted_iota(i32, (128, 128), 1)
    ang = ((ri * ci) & 127).astype(f32) * (2 * math.pi / 128)
    cb, sb = jnp.cos(ang), jnp.sin(ang)
    ang = (ri[0:16] * ci[0:16]).astype(f32) * (2 * math.pi / S)
    ct_all, st_all = jnp.cos(ang) * _SCALE, jnp.sin(ang) * _SCALE

    def rotated(rows, a):
        ct, st = ct_all[a:a + 1], st_all[a:a + 1]
        return cb[0:rows] * ct - sb[0:rows] * st, sb[0:rows] * ct + cb[0:rows] * st

    def store(m, c, s):
        m[0], m[1], m[2] = c.astype(bf16), (-(c + s)).astype(bf16), (s - c).astype(bf16)

    for p in range(4):
        c0, s0 = rotated(64, 2 * p)
        c1, s1 = rotated(64, 2 * (4 if p == 0 else 8 - p))
        if p == 0:
            nyquist = jnp.where((ci[0:64] & 1) == 0, _SCALE, -_SCALE)
            s0 = jnp.where(ri[0:64] == 0, nyquist, -s0)
            m1[0, 0] = jnp.concatenate([c0, s0], axis=0).astype(bf16)
            m1[0, 1] = jnp.concatenate([c1, -s1], axis=0).astype(bf16)
        else:
            store(m1.at[p], jnp.concatenate([c0, c1], axis=0), jnp.concatenate([s0, -s1], axis=0))

    return lambda a: store(m2.at[a], *rotated(128, a))


def _forward(xv, m1, m2, gbuf, wait_x, build_m2, late_work):
    sub = lax.broadcasted_iota(i32, (8, 128), 0)
    inputs = {}

    def butterflies(a, quarter):
        extract = (_lo_f32, _hi_f32)[a % 2]
        for g in range(2 * quarter, 2 * quarter + 2):
            u = _rfft8([extract(xv[a // 2, g * 16:(g + 1) * 16, j * 128:(j + 1) * 128])
                        for j in range(8)])
            for p in range(4):
                parts = u[p] if p == 0 else (*u[p], u[p][0] + u[p][1])
                for k, part in enumerate(parts):
                    inputs.setdefault((a, p, k), []).append(part)

    def feature_stage(a, p):
        u = [jnp.concatenate(inputs.pop((a, p, k)), axis=0).astype(bf16)
             for k in range(3 if p else 2)]
        if p > 0:
            tr, ti = _complex_product(_from_left, m1.at[p], *u, True)
            return tr, jnp.concatenate([ti[0:64], -ti[64:128]], axis=0)
        t0, t1 = [_from_left(_halves(m1[0, k]), u[k]) for k in range(2)]
        tr = [jnp.where(sub == 0, t0[0:8] * 0.5, t0[0:8]), t0[8:64], t1[0:64],
              jnp.where(sub == 0, t0[64:72] * 0.5, 0.0)]
        ti = [jnp.where(sub == 0, 0.0, t0[64:72]), t0[72:128], t1[64:128],
              jnp.zeros((8, 128), f32)]
        return jnp.concatenate(tr, axis=0), jnp.concatenate(ti, axis=0)

    def sequence_stage(a, p, t):
        for k, g in enumerate(_complex_product(_from_right, m2.at[a], *t, t[0] + t[1], True)):
            for blk in range(16):
                gbuf[p * 16 + blk, a, :, k * 128:(k + 1) * 128] = g[blk * 8:(blk + 1) * 8]
            if p == 0:
                gbuf[64, a, :, k * 128:(k + 1) * 128] = g[128:136]

    build_m2(0)
    build_m2(1)
    wait_x(0)
    for quarter in range(4):
        butterflies(0, quarter)
    pending = None
    for i in range(64):
        a, p = divmod(i, 4)
        t = feature_stage(a, p)
        if a < 15:
            if p == 0 and a % 2 == 1:
                wait_x((a + 1) // 2)
            butterflies(a + 1, p)
        if p == 1 and a < 14:
            build_m2(a + 2)
        if i >= 44:
            next(late_work, None)
        if pending is not None:
            sequence_stage(*pending)
        pending = (a, p, t)
    sequence_stage(*pending)


def _filter_rows(g, gbuf, filt=None):
    def load(slots):
        return [(gbuf[g, a, :, 0:128], gbuf[g, a, :, 128:256]) for a in slots]

    def store(slots, values):
        for a, (re, im) in zip(slots, values):
            gbuf[g, a, :, 0:128] = re
            gbuf[g, a, :, 128:256] = im

    if filt is None:
        for a0 in range(4):
            slots = range(a0, 16, 4)
            ys = _fft4(*load(slots), -1)
            store(slots, [_twiddle16(ys[k0], a0 * k0, -1) for k0 in range(4)])
            yield
        return
    for k0 in range(4):
        slots = range(4 * k0, 4 * k0 + 4)
        ys = []
        for k1, (xr, xi) in enumerate(_fft4(*load(slots), -1)):
            wr, wi = filt(k0 + 4 * k1)
            ys.append((xr * wr - xi * wi, xr * wi + xi * wr))
        ys = _fft4(*ys, +1)
        store(slots, [_twiddle16(ys[a0], a0 * k0, +1) for a0 in range(4)])
        yield
    for a0 in range(4):
        slots = range(a0, 16, 4)
        store(slots, _fft4(*load(slots), +1))
        yield


def _inverse(m1, m2, gbuf, rbuf, yv, other_work):
    sub = lax.broadcasted_iota(i32, (8, 128), 0)
    sign = jnp.where(lax.broadcasted_iota(i32, (128, 128), 1) < 64, 1.0, -1.0)

    def sequence_stage(a, p):
        hr, hi = [gbuf[p * 16:(p + 1) * 16, a, :, k * 128:(k + 1) * 128].reshape(128, 128)
                  for k in range(2)]
        if p > 0:
            zr, zi = _complex_product(_from_left, m2.at[a], hr.astype(bf16), hi.astype(bf16),
                                      (hr + hi).astype(bf16), False)
            return zr, zi * sign
        nr, ni = gbuf[64, a, :, 0:128], gbuf[64, a, :, 128:256]
        low = ([hr[0:64], jnp.where(sub == 0, nr, hi[0:8]), hi[8:64]],
               [hi[0:64], jnp.where(sub == 0, ni, -hr[0:8]), -hr[8:64]])
        high = ([hr[64:128], hi[64:128]], [hi[64:128], -hr[64:128]])
        zs = []
        for re, im in (low, high):
            re, im = jnp.concatenate(re, axis=0), jnp.concatenate(im, axis=0)
            zs.append(_from_left(_halves(m2[a, 1]), im.astype(bf16))
                      + _from_left(_halves(m2[a, 0]), (re + im).astype(bf16)))
        return zs

    def feature_stage(a, p, z):
        if p > 0:
            v = _complex_product(_from_right, m1.at[p], *z, z[0] + z[1], False)
        else:
            v = [_from_right(_halves(m1[0, k]), z[k]) for k in range(2)]
        rbuf[a % 4, p, 0] = v[0]
        rbuf[a % 4, p, 1] = v[1]

    def butterflies(r, eighth):
        for g in range(2 * eighth, 2 * eighth + 2):
            rows = slice(g * 8, (g + 1) * 8)
            ys = [_irfft8(*[(rbuf[a % 4, p, 0, rows, :], rbuf[a % 4, p, 1, rows, :])
                            for p in range(4)]) for a in (2 * r, 2 * r + 1)]
            for j in range(8):
                even = pltpu.bitcast(ys[0][j].astype(bf16).astype(f32), i32)
                odd = pltpu.bitcast(ys[1][j].astype(bf16).astype(f32), i32)
                yv[r, rows, j * 128:(j + 1) * 128] = lax.shift_right_logical(even, 16) | odd

    pending = {}
    for i in range(64 + 9):
        if i < 64:
            pending[i] = sequence_stage(*divmod(i, 4))
            next(other_work, None)
        if 1 <= i <= 64:
            feature_stage(*divmod(i - 1, 4), pending.pop(i - 1))
        if i >= 9:
            butterflies(*divmod(i - 9, 8))


def _interleave_heads(w, items, pieces=1):
    per_piece = D // 16 // pieces
    for first in range(0, D // 16, per_piece):
        for i in items:
            for c in range(first, first + per_piece, 2):
                even, odd = w[i, c:c + 2, 0], w[i, c:c + 2, 1]
                w[i, c:c + 2, 0] = (even & 0xFFFF) | (odd << 16)
                w[i, c:c + 2, 1] = lax.shift_right_logical(even, 16) | (odd & _HI16)
        yield


def _head_weight(w, i, e):
    return _halves(w[i, :, e].reshape(D // 2, DH))


def _segment(s, wqkv, wo32, xs, early_rows, h_ref, outs):
    z0 = pl.multiple_of(s * 8, 8)
    h_ref[M:L, :] = xs[s].astype(f32)
    row = lax.broadcasted_iota(i32, (L, L), 0)
    col = lax.broadcasted_iota(i32, (L, L), 1)
    mask = (row < M) | (row >= col)

    def project(h):
        items = [m * NPAIR + h // 2 for m in range(3)]
        ws = [_head_weight(wqkv, i, h % 2) for i in items]
        rows = [L - 8 if i < EARLY_ITEMS else L for i in items]
        if h == 0:
            first = [_dot(h_ref[0:n, 0:D // 2], w[0:D // 2]) for n, w in zip(rows, ws)]
            qkv = [_dot(h_ref[0:n, D // 2:D], w[D // 2:D]) + f for n, w, f in zip(rows, ws, first)]
        else:
            qkv = [_dot(h_ref[0:n, :], w) for n, w in zip(rows, ws)]
        return [jnp.concatenate([v, early_rows[2 * i + h % 2, pl.ds(z0, 8), :]], axis=0)
                if i < EARLY_ITEMS else v for v, i in zip(qkv, items)]

    def probabilities(q, k):
        sc = _dot(q, k.astype(bf16), _NT) * DH ** -0.5
        sc = jnp.where(mask, sc, -1e9)
        e = jnp.exp(sc - jnp.max(sc, axis=-1, keepdims=True))
        return e * pltpu.reciprocal(jnp.sum(e, axis=-1, keepdims=True), approx=False)

    def out_proj(o, n, lo, hi):
        w = _halves(wo32[n, lo * DH // 2:hi * DH // 2, :])
        return _dot(jnp.concatenate(o[lo:hi], axis=1), w)

    lag_scores, lag_mix, split = 2, 4, 24
    state, o, part = {}, [None] * H, [None] * 8
    for t in range(H + 8):
        if t < H:
            state[t] = project(t)
        else:
            part[t - H] = out_proj(o, t - H, 0, split)
        if 0 <= t - lag_scores < H:
            q, k, v = state[t - lag_scores]
            state[t - lag_scores] = (probabilities(q, k), v)
        if 0 <= t - lag_mix < H:
            p, v = state.pop(t - lag_mix)
            o[t - lag_mix] = _dot(p, v.astype(bf16))
    for n in range(8):
        res = out_proj(o, n, split, H) + part[n]
        h_ref[0:M, n * 128:(n + 1) * 128] = res[0:M]
        for i in range(SEG // 16):
            outs[2 * s + i, :, n * 128:(n + 1) * 128] = res[M + 16 * i:M + 16 * i + 16].astype(bf16)


def _kernel(ax_hbm, wr_hbm, wi_hbm, bx_hbm, mem0_hbm, wq_hbm, wk_hbm, wv_hbm, wo_hbm, out_hbm,
            xv, wrv, wiv, wnr, wni, m1, m2, gbuf, rbuf, yv,
            wqkv, wo, xs, xz_raw, xz, early_rows, mem0_ref, h_ref, outs,
            sem_ax, sem_f, sem_w, sem_wo, sem_bx, sem_xz, sem_ya, sem_yb):
    ax32 = ax_hbm.bitcast(i32)
    out32 = out_hbm.bitcast(i32)

    def ax_copy(r):
        return pltpu.make_async_copy(ax32.at[:, r, :], xv.at[r], sem_ax.at[r])

    def ya_copy(r):
        return pltpu.make_async_copy(yv.at[r], out32.at[:, r, pl.ds(0, D)], sem_ya.at[0])

    def bx_copy(c):
        return pltpu.make_async_copy(bx_hbm.at[pl.ds(c * SCHUNK, SCHUNK)],
                                     xs.at[pl.ds(c * SCHUNK, SCHUNK)], sem_bx.at[c])

    def yb_copy(c):
        rows = pl.ds(c * (SCHUNK * SEG // 16), SCHUNK * SEG // 16)
        return pltpu.make_async_copy(outs.at[rows], out_hbm.at[rows, :, pl.ds(D, D)], sem_yb.at[0])

    f_copies = [pltpu.make_async_copy(src.at[pl.ds(0, D // 2), pl.ds(k1 * 128, 128)],
                                      dst.at[k1, pl.ds(0, D // 4)].bitcast(bf16), sem_f.at[0])
                for k1 in range(16) for src, dst in ((wr_hbm, wrv), (wi_hbm, wiv))]
    f_copies += [pltpu.make_async_copy(src.at[pl.ds(D // 2, 1), :], dst, sem_f.at[0])
                 for src, dst in ((wr_hbm, wnr), (wi_hbm, wni))]
    wo_copies = [pltpu.make_async_copy(wo_hbm.at[:, pl.ds(n * 128, 128)], wo.at[n], sem_wo.at[0])
                 for n in range(8)]
    wo_copies.append(pltpu.make_async_copy(mem0_hbm, mem0_ref, sem_wo.at[0]))

    def start_pair(m, j):
        w32 = (wq_hbm, wk_hbm, wv_hbm)[m].bitcast(i32)
        for e in range(2):
            pltpu.make_async_copy(w32.at[:, :, e, j, :], wqkv.at[m * NPAIR + j, :, e],
                                  sem_w.at[m * NPAIR + j]).start()

    def wait_item(i):
        pltpu.make_async_copy(wqkv.at[i], wqkv.at[i], sem_w.at[i]).wait()

    for r in range(8):
        ax_copy(r).start()
    xz_copy = pltpu.make_async_copy(bx_hbm.at[:, pl.ds(SEG - 8, 8), :], xz_raw, sem_xz.at[0])
    xz_copy.start()
    for j in range(FIRST_ITEMS + 2):
        start_pair(0, j)
    for cp in f_copies:
        cp.start()

    build_m2 = _build_dft_matrices(m1, m2)

    def wait_x(r):
        for i in {0: (0,), 1: (1, 2), 3: (3, 4, 5), 6: (6, 7)}.get(r, ()):
            ax_copy(i).wait()
        if r == 6:
            xz_copy.wait()
            for i in range(2):
                wait_item(i)

    def prepare_early():
        interleave = _interleave_heads(wqkv, (0, 1), 16)
        for c in range(0, NSEG, 4):
            xz[c * 8:(c + 4) * 8, :] = xz_raw[c:c + 4].astype(f32).reshape(32, D)
            next(interleave)
            yield

    m1, m2 = m1.bitcast(i32), m2.bitcast(i32)
    _forward(xv, m1, m2, gbuf, wait_x, build_m2, prepare_early())

    for j in range(FIRST_ITEMS + 2, NPAIR):
        start_pair(0, j)
    for j in range(8):
        start_pair(1, j)

    def filter_groups(t):
        for k1 in range(8):
            extract = (_lo_f32, _hi_f32)[k1 % 2]
            g = t + (16 * k1 if k1 < 4 else 16 * ((8 - k1) % 4) + 8)
            yield from _filter_rows(g, gbuf, lambda k: tuple(
                extract(w[k, pl.ds(32 * t + k1 // 2, 8, stride=4), :]) for w in (wrv, wiv)))

    def project_early(items, interleave_work, filter_work=iter(()), pieces=lambda n: 0):
        for n, (i, e, r0) in enumerate((i, e, r0) for i in items for e in range(2)
                                       for r0 in range(0, NSEG * 8, 64)):
            res = _dot(xz[r0:r0 + 64, :], _head_weight(wqkv, i, e))
            early_rows[2 * i + e, r0:r0 + 64, :] = res
            gbuf[65 + i % 2, 0, :, 0:128] = res[56:64]
            next(interleave_work, None)
            for _ in range(pieces(n)):
                next(filter_work, None)

    @pl.loop(0, FIRST_ITEMS)
    def _(i):
        wait_item(i + 2)
        filter_work = (x for n in range(13) for x in _filter_rows(13 * i + n, gbuf))
        project_early((i,), _interleave_heads(wqkv, (i + 2,), 16),
                      filter_work, lambda n: 4 if n % 2 == 0 else 3)

    for j in range(8, NPAIR):
        start_pair(1, j)
    for cp in f_copies:
        cp.wait()

    @pl.loop(0, 4)
    def _(u):
        for i in range(4):
            start_pair(2, 4 * u + i)

        @pl.loop(2 * u, 2 * u + 2)
        def _(t):
            ahead = (FIRST_ITEMS + 2 * t + 2, FIRST_ITEMS + 2 * t + 3)
            for i in ahead:
                wait_item(i)
            project_early((FIRST_ITEMS + 2 * t, FIRST_ITEMS + 2 * t + 1),
                          _interleave_heads(wqkv, ahead, 32),
                          filter_groups(t), lambda n: 3 if n % 8 == 0 else 2)

    bx_copy(0).start()
    for cp in wo_copies:
        cp.start()
    list(_filter_rows(64, gbuf, lambda k: tuple(
        jnp.broadcast_to(w[:, k * 128:(k + 1) * 128].astype(f32), (8, 128)) for w in (wnr, wni))))

    done = FIRST_ITEMS + 16
    for i in range(done + 2, 2 * NPAIR):
        wait_item(i)
    _inverse(m1, m2, gbuf, rbuf, yv, _interleave_heads(wqkv, range(done + 2, 2 * NPAIR), 32))

    steps = EARLY_ITEMS - done
    per_step = NPAIR // steps
    assert per_step * steps == NPAIR
    for i in range(2 * NPAIR, 3 * NPAIR):
        wait_item(i)

    @pl.loop(0, steps)
    def _(t):
        ahead = [2 * NPAIR + per_step * t + i for i in range(per_step)]
        project_early((done + t,), _interleave_heads(wqkv, ahead, 16))

    for cp in wo_copies:
        cp.wait()
    for c in range(1, NCHUNK):
        bx_copy(c).start()
    for r in range(8):
        ya_copy(r).start()
    h_ref[0:M, :] = mem0_ref[...].astype(f32)
    wo32 = wo.bitcast(i32)

    @pl.loop(0, NCHUNK)
    def _(c):
        bx_copy(c).wait()
        for i in range(SCHUNK):
            _segment(c * SCHUNK + i, wqkv, wo32, xs, early_rows, h_ref, outs)
        yb_copy(c).start()

    for r in range(8):
        ya_copy(r).wait()
    for c in range(NCHUNK):
        yb_copy(c).wait()


@functools.partial(jax.jit, static_argnames=("B_seg_len",))
def pallas_concat_heads__spectral_gfnet__memory_aug_recurrent_mem_tr__prompt_kernel(
    A_x, A_w_r, A_w_i, B_x, B_mem0, B_Wq, B_Wk, B_Wv, B_Wo, B_seg_len,
):
    assert A_x.shape == (1, S, D) and B_x.shape == (1, S, D) and B_mem0.shape == (1, M, D)
    assert A_w_r.shape == (S, D // 2 + 1) and B_Wq.shape == (D, H, DH) and B_Wo.shape == (H, DH, D)
    assert B_seg_len == SEG
    hbm = pl.BlockSpec(memory_space=pl.ANY)
    out = pl.pallas_call(
        _kernel,
        out_shape=jax.ShapeDtypeStruct((S // 16, 16, 2 * D), bf16),
        in_specs=[hbm] * 9,
        out_specs=hbm,
        scratch_shapes=[
            pltpu.VMEM((8, 128, D), i32),
            pltpu.VMEM((16, D // 4 + 8, 128), i32),
            pltpu.VMEM((16, D // 4 + 8, 128), i32),
            pltpu.VMEM((1, S), bf16),
            pltpu.VMEM((1, S), bf16),
            pltpu.VMEM((4, 3, 128, 128), bf16),
            pltpu.VMEM((16, 3, 128, 128), bf16),
            pltpu.VMEM((67, 16, 8, 256), f32),
            pltpu.VMEM((4, 4, 2, 128, 128), f32),
            pltpu.VMEM((8, 128, D), i32),
            pltpu.VMEM((3 * NPAIR, D // 16, 2, 8, DH), i32),
            pltpu.VMEM((8, H * DH, 128), bf16),
            pltpu.VMEM((NSEG, SEG, D), bf16),
            pltpu.VMEM((NSEG, 8, D), bf16),
            pltpu.VMEM((NSEG * 8, D), f32),
            pltpu.VMEM((2 * EARLY_ITEMS, NSEG * 8, DH), f32),
            pltpu.VMEM((M, D), bf16),
            pltpu.VMEM((L, D), f32),
            pltpu.VMEM((S // 16, 16, D), bf16),
            pltpu.SemaphoreType.DMA((8,)),
            pltpu.SemaphoreType.DMA((1,)),
            pltpu.SemaphoreType.DMA((3 * NPAIR,)),
            pltpu.SemaphoreType.DMA((1,)),
            pltpu.SemaphoreType.DMA((NCHUNK,)),
            pltpu.SemaphoreType.DMA((1,)),
            pltpu.SemaphoreType.DMA((1,)),
            pltpu.SemaphoreType.DMA((1,)),
        ],
        compiler_params=pltpu.CompilerParams(vmem_limit_bytes=100 * 1024 * 1024),
    )(
        A_x.reshape(S // 16, 16, D), A_w_r.T, A_w_i.T,
        B_x.reshape(NSEG, SEG, D), B_mem0.reshape(M, D),
        B_Wq.reshape(D // 16, 8, 2, H, DH), B_Wk.reshape(D // 16, 8, 2, H, DH),
        B_Wv.reshape(D // 16, 8, 2, H, DH), B_Wo.reshape(H * DH, D),
    )
    return out.reshape(1, S, 2 * D)
```

```python
import functools
import math

import jax
import jax.numpy as jnp
from jax import lax
import jax.experimental.pallas as pl
import jax.experimental.pallas.tpu as pltpu

bf16, f32, i32 = jnp.bfloat16, jnp.float32, jnp.int32

S, D = 2048, 1024
H, DH = 32, 128
M, SEG = 8, 32
L = M + SEG
NSEG = S // SEG
NPAIR = H // 2
FIRST_ITEMS = 5
EARLY_ITEMS = 25
SCHUNK = 2
NCHUNK = NSEG // SCHUNK

_NN = (((1,), (0,)), ((), ()))
_NT = (((1,), (1,)), ((), ()))
_HI16 = -65536
_R2 = math.sqrt(0.5)
_SCALE = 2.0 ** -5


def _dot(a, b, dims=_NN):
    return lax.dot_general(a, b, dims, preferred_element_type=f32)


def _lo_f32(w):
    return pltpu.bitcast(w << 16, f32)


def _hi_f32(w):
    return pltpu.bitcast(w & _HI16, f32)


def _cadd(a, b):
    return a[0] + b[0], a[1] + b[1]


def _csub(a, b):
    return a[0] - b[0], a[1] - b[1]


def _fft4(x0, x1, x2, x3, sign):
    a, b = _cadd(x0, x2), _csub(x0, x2)
    c, d = _cadd(x1, x3), _csub(x1, x3)
    minus_i = (b[0] + d[1], b[1] - d[0])
    plus_i = (b[0] - d[1], b[1] + d[0])
    if sign < 0:
        return _cadd(a, c), minus_i, _csub(a, c), plus_i
    return _cadd(a, c), plus_i, _csub(a, c), minus_i


def _twiddle16(x, m, sign):
    if m == 0:
        return x
    if m == 4:
        return (-x[1], x[0]) if sign > 0 else (x[1], -x[0])
    if m == 2:
        if sign > 0:
            return (x[0] - x[1]) * _R2, (x[0] + x[1]) * _R2
        return (x[0] + x[1]) * _R2, (x[1] - x[0]) * _R2
    if m == 6:
        if sign > 0:
            return (x[0] + x[1]) * -_R2, (x[0] - x[1]) * _R2
        return (x[1] - x[0]) * _R2, (x[0] + x[1]) * -_R2
    c, s = math.cos(2 * math.pi * m / 16), sign * math.sin(2 * math.pi * m / 16)
    return x[0] * c - x[1] * s, x[0] * s + x[1] * c


def _rfft8(x):
    s04, d04 = x[0] + x[4], x[0] - x[4]
    s26, d26 = x[2] + x[6], x[2] - x[6]
    s15, d15 = x[1] + x[5], x[1] - x[5]
    s37, d37 = x[3] + x[7], x[3] - x[7]
    e, o = s04 + s26, s15 + s37
    p, q = (d15 - d37) * _R2, (d15 + d37) * _R2
    return (e + o, e - o), (d04 + p, -(d26 + q)), (s04 - s26, s37 - s15), (d04 - p, d26 - q)


def _irfft8(r0, r1, r2, r3):
    a0, a4 = r0[0] + r0[1], r0[0] - r0[1]
    e0, e2 = a0 + r2[0], a0 - r2[0]
    e1, e3 = a4 - r2[1], a4 + r2[1]
    o0, o2 = r1[0] + r3[0], r3[1] - r1[1]
    dr, si = r1[0] - r3[0], r1[1] + r3[1]
    o1, o3 = (dr - si) * _R2, (dr + si) * -_R2
    return [e0 + o0, e1 + o1, e2 + o2, e3 + o3, e0 - o0, e1 - o1, e2 - o2, e3 - o3]


def _halves(w):
    return pltpu.bitcast(w, bf16)


def _complex_product(apply, m, xr, xi, xs, conjugate):
    shared = apply(_halves(m[0]), xs)
    for_re, for_im = (2, 1) if conjugate else (1, 2)
    return apply(_halves(m[for_re]), xi) + shared, apply(_halves(m[for_im]), xr) + shared


def _from_left(m, x):
    return _dot(m, x, _NT)


def _from_right(m, x):
    return _dot(x, m)


def _build_dft_matrices(m1, m2):
    ri = lax.broadcasted_iota(i32, (128, 128), 0)
    ci = lax.broadcasted_iota(i32, (128, 128), 1)
    ang = ((ri * ci) & 127).astype(f32) * (2 * math.pi / 128)
    cb, sb = jnp.cos(ang), jnp.sin(ang)
    ang = (ri[0:16] * ci[0:16]).astype(f32) * (2 * math.pi / S)
    ct_all, st_all = jnp.cos(ang) * _SCALE, jnp.sin(ang) * _SCALE

    def rotated(rows, a):
        ct, st = ct_all[a:a + 1], st_all[a:a + 1]
        return cb[0:rows] * ct - sb[0:rows] * st, sb[0:rows] * ct + cb[0:rows] * st

    def store(m, c, s):
        m[0], m[1], m[2] = c.astype(bf16), (-(c + s)).astype(bf16), (s - c).astype(bf16)

    for p in range(4):
        c0, s0 = rotated(64, 2 * p)
        c1, s1 = rotated(64, 2 * (4 if p == 0 else 8 - p))
        if p == 0:
            nyquist = jnp.where((ci[0:64] & 1) == 0, _SCALE, -_SCALE)
            s0 = jnp.where(ri[0:64] == 0, nyquist, -s0)
            m1[0, 0] = jnp.concatenate([c0, s0], axis=0).astype(bf16)
            m1[0, 1] = jnp.concatenate([c1, -s1], axis=0).astype(bf16)
        else:
            store(m1.at[p], jnp.concatenate([c0, c1], axis=0), jnp.concatenate([s0, -s1], axis=0))

    for a in range(16):
        store(m2.at[a], *rotated(128, a))


def _forward(xv, m1, m2, gbuf, wait_x, late_work):
    sub = lax.broadcasted_iota(i32, (8, 128), 0)
    inputs = {}

    def butterflies(a, quarter):
        extract = (_lo_f32, _hi_f32)[a % 2]
        for g in range(2 * quarter, 2 * quarter + 2):
            u = _rfft8([extract(xv[a // 2, g * 16:(g + 1) * 16, j * 128:(j + 1) * 128])
                        for j in range(8)])
            for p in range(4):
                parts = u[p] if p == 0 else (*u[p], u[p][0] + u[p][1])
                for k, part in enumerate(parts):
                    inputs.setdefault((a, p, k), []).append(part)

    def feature_stage(a, p):
        u = [jnp.concatenate(inputs.pop((a, p, k)), axis=0).astype(bf16)
             for k in range(3 if p else 2)]
        if p > 0:
            tr, ti = _complex_product(_from_left, m1.at[p], *u, True)
            return tr, jnp.concatenate([ti[0:64], -ti[64:128]], axis=0)
        t0, t1 = [_from_left(_halves(m1[0, k]), u[k]) for k in range(2)]
        tr = [jnp.where(sub == 0, t0[0:8] * 0.5, t0[0:8]), t0[8:64], t1[0:64],
              jnp.where(sub == 0, t0[64:72] * 0.5, 0.0)]
        ti = [jnp.where(sub == 0, 0.0, t0[64:72]), t0[72:128], t1[64:128],
              jnp.zeros((8, 128), f32)]
        return jnp.concatenate(tr, axis=0), jnp.concatenate(ti, axis=0)

    def sequence_stage(a, p, t):
        for k, g in enumerate(_complex_product(_from_right, m2.at[a], *t, t[0] + t[1], True)):
            for blk in range(16):
                gbuf[p * 16 + blk, a, :, k * 128:(k + 1) * 128] = g[blk * 8:(blk + 1) * 8]
            if p == 0:
                gbuf[64, a, :, k * 128:(k + 1) * 128] = g[128:136]

    wait_x(0)
    for quarter in range(4):
        butterflies(0, quarter)
    pending = None
    for i in range(64):
        a, p = divmod(i, 4)
        t = feature_stage(a, p)
        if a < 15:
            if p == 0 and a % 2 == 1:
                wait_x((a + 1) // 2)
            butterflies(a + 1, p)
        if i >= 44:
            next(late_work, None)
        if pending is not None:
            sequence_stage(*pending)
        pending = (a, p, t)
    sequence_stage(*pending)


def _filter_rows(g, gbuf, filt=None):
    def load(slots):
        return [(gbuf[g, a, :, 0:128], gbuf[g, a, :, 128:256]) for a in slots]

    def store(slots, values):
        for a, (re, im) in zip(slots, values):
            gbuf[g, a, :, 0:128] = re
            gbuf[g, a, :, 128:256] = im

    if filt is None:
        for a0 in range(4):
            slots = range(a0, 16, 4)
            ys = _fft4(*load(slots), -1)
            store(slots, [_twiddle16(ys[k0], a0 * k0, -1) for k0 in range(4)])
            yield
        return
    for k0 in range(4):
        slots = range(4 * k0, 4 * k0 + 4)
        ys = []
        for k1, (xr, xi) in enumerate(_fft4(*load(slots), -1)):
            wr, wi = filt(k0 + 4 * k1)
            ys.append((xr * wr - xi * wi, xr * wi + xi * wr))
        ys = _fft4(*ys, +1)
        store(slots, [_twiddle16(ys[a0], a0 * k0, +1) for a0 in range(4)])
        yield
    for a0 in range(4):
        slots = range(a0, 16, 4)
        store(slots, _fft4(*load(slots), +1))
        yield


def _inverse(m1, m2, gbuf, rbuf, yv, other_work):
    sub = lax.broadcasted_iota(i32, (8, 128), 0)
    sign = jnp.where(lax.broadcasted_iota(i32, (128, 128), 1) < 64, 1.0, -1.0)

    def sequence_stage(a, p):
        hr, hi = [gbuf[p * 16:(p + 1) * 16, a, :, k * 128:(k + 1) * 128].reshape(128, 128)
                  for k in range(2)]
        if p > 0:
            zr, zi = _complex_product(_from_left, m2.at[a], hr.astype(bf16), hi.astype(bf16),
                                      (hr + hi).astype(bf16), False)
            return zr, zi * sign
        nr, ni = gbuf[64, a, :, 0:128], gbuf[64, a, :, 128:256]
        low = ([hr[0:64], jnp.where(sub == 0, nr, hi[0:8]), hi[8:64]],
               [hi[0:64], jnp.where(sub == 0, ni, -hr[0:8]), -hr[8:64]])
        high = ([hr[64:128], hi[64:128]], [hi[64:128], -hr[64:128]])
        zs = []
        for re, im in (low, high):
            re, im = jnp.concatenate(re, axis=0), jnp.concatenate(im, axis=0)
            zs.append(_from_left(_halves(m2[a, 1]), im.astype(bf16))
                      + _from_left(_halves(m2[a, 0]), (re + im).astype(bf16)))
        return zs

    def feature_stage(a, p, z):
        if p > 0:
            v = _complex_product(_from_right, m1.at[p], *z, z[0] + z[1], False)
        else:
            v = [_from_right(_halves(m1[0, k]), z[k]) for k in range(2)]
        rbuf[a % 4, p, 0] = v[0]
        rbuf[a % 4, p, 1] = v[1]

    def butterflies(r, eighth):
        for g in range(2 * eighth, 2 * eighth + 2):
            rows = slice(g * 8, (g + 1) * 8)
            ys = [_irfft8(*[(rbuf[a % 4, p, 0, rows, :], rbuf[a % 4, p, 1, rows, :])
                            for p in range(4)]) for a in (2 * r, 2 * r + 1)]
            for j in range(8):
                even = pltpu.bitcast(ys[0][j].astype(bf16).astype(f32), i32)
                odd = pltpu.bitcast(ys[1][j].astype(bf16).astype(f32), i32)
                yv[r, rows, j * 128:(j + 1) * 128] = lax.shift_right_logical(even, 16) | odd

    pending = {}
    for i in range(64 + 9):
        if i < 64:
            pending[i] = sequence_stage(*divmod(i, 4))
            next(other_work, None)
        if 1 <= i <= 64:
            feature_stage(*divmod(i - 1, 4), pending.pop(i - 1))
        if i >= 9:
            butterflies(*divmod(i - 9, 8))


def _interleave_heads(w, items, pieces=1):
    per_piece = D // 16 // pieces
    for first in range(0, D // 16, per_piece):
        for i in items:
            for c in range(first, first + per_piece, 2):
                even, odd = w[i, c:c + 2, 0], w[i, c:c + 2, 1]
                w[i, c:c + 2, 0] = (even & 0xFFFF) | (odd << 16)
                w[i, c:c + 2, 1] = lax.shift_right_logical(even, 16) | (odd & _HI16)
        yield


def _head_weight(w, i, e):
    return _halves(w[i, :, e].reshape(D // 2, DH))


def _segment(s, wqkv, wo32, xs, early_rows, h_ref, outs):
    z0 = pl.multiple_of(s * 8, 8)
    h_ref[M:L, :] = xs[s].astype(f32)
    row = lax.broadcasted_iota(i32, (L, L), 0)
    col = lax.broadcasted_iota(i32, (L, L), 1)
    mask = (row < M) | (row >= col)

    def project(h):
        items = [m * NPAIR + h // 2 for m in range(3)]
        ws = [_head_weight(wqkv, i, h % 2) for i in items]
        rows = [L - 8 if i < EARLY_ITEMS else L for i in items]
        if h == 0:
            first = [_dot(h_ref[0:n, 0:D // 2], w[0:D // 2]) for n, w in zip(rows, ws)]
            qkv = [_dot(h_ref[0:n, D // 2:D], w[D // 2:D]) + f for n, w, f in zip(rows, ws, first)]
        else:
            qkv = [_dot(h_ref[0:n, :], w) for n, w in zip(rows, ws)]
        return [jnp.concatenate([v, early_rows[2 * i + h % 2, pl.ds(z0, 8), :]], axis=0)
                if i < EARLY_ITEMS else v for v, i in zip(qkv, items)]

    def probabilities(q, k):
        sc = _dot(q, k.astype(bf16), _NT) * DH ** -0.5
        sc = jnp.where(mask, sc, -1e9)
        e = jnp.exp(sc - jnp.max(sc, axis=-1, keepdims=True))
        return e * pltpu.reciprocal(jnp.sum(e, axis=-1, keepdims=True), approx=False)

    def out_proj(o, n, lo, hi):
        w = _halves(wo32[n, lo * DH // 2:hi * DH // 2, :])
        return _dot(jnp.concatenate(o[lo:hi], axis=1), w)

    lag_scores, lag_mix, split = 2, 4, 24
    state, o, part = {}, [None] * H, [None] * 8
    for t in range(H + 8):
        if t < H:
            state[t] = project(t)
        else:
            part[t - H] = out_proj(o, t - H, 0, split)
        if 0 <= t - lag_scores < H:
            q, k, v = state[t - lag_scores]
            state[t - lag_scores] = (probabilities(q, k), v)
        if 0 <= t - lag_mix < H:
            p, v = state.pop(t - lag_mix)
            o[t - lag_mix] = _dot(p, v.astype(bf16))
    for n in range(8):
        res = out_proj(o, n, split, H) + part[n]
        h_ref[0:M, n * 128:(n + 1) * 128] = res[0:M]
        for i in range(SEG // 16):
            outs[2 * s + i, :, n * 128:(n + 1) * 128] = res[M + 16 * i:M + 16 * i + 16].astype(bf16)


def _kernel(ax_hbm, wr_hbm, wi_hbm, bx_hbm, mem0_hbm, wq_hbm, wk_hbm, wv_hbm, wo_hbm, out_hbm,
            xv, wrv, wiv, wnr, wni, m1, m2, gbuf, rbuf, yv,
            wqkv, wo, xs, xz_raw, xz, early_rows, mem0_ref, h_ref, outs,
            sem_ax, sem_f, sem_w, sem_wo, sem_bx, sem_xz, sem_ya, sem_yb):
    ax32 = ax_hbm.bitcast(i32)
    out32 = out_hbm.bitcast(i32)

    def ax_copy(r):
        return pltpu.make_async_copy(ax32.at[:, r, :], xv.at[r], sem_ax.at[r])

    def ya_copy(r):
        return pltpu.make_async_copy(yv.at[r], out32.at[:, r, pl.ds(0, D)], sem_ya.at[0])

    def bx_copy(c):
        return pltpu.make_async_copy(bx_hbm.at[pl.ds(c * SCHUNK, SCHUNK)],
                                     xs.at[pl.ds(c * SCHUNK, SCHUNK)], sem_bx.at[c])

    def yb_copy(c):
        rows = pl.ds(c * (SCHUNK * SEG // 16), SCHUNK * SEG // 16)
        return pltpu.make_async_copy(outs.at[rows], out_hbm.at[rows, :, pl.ds(D, D)], sem_yb.at[0])

    f_copies = [pltpu.make_async_copy(src.at[pl.ds(0, D // 2), pl.ds(k1 * 128, 128)],
                                      dst.at[k1, pl.ds(0, D // 4)].bitcast(bf16), sem_f.at[0])
                for k1 in range(16) for src, dst in ((wr_hbm, wrv), (wi_hbm, wiv))]
    f_copies += [pltpu.make_async_copy(src.at[pl.ds(D // 2, 1), :], dst, sem_f.at[0])
                 for src, dst in ((wr_hbm, wnr), (wi_hbm, wni))]
    wo_copies = [pltpu.make_async_copy(wo_hbm.at[:, pl.ds(n * 128, 128)], wo.at[n], sem_wo.at[0])
                 for n in range(8)]
    wo_copies.append(pltpu.make_async_copy(mem0_hbm, mem0_ref, sem_wo.at[0]))

    def start_pair(m, j):
        w32 = (wq_hbm, wk_hbm, wv_hbm)[m].bitcast(i32)
        for e in range(2):
            pltpu.make_async_copy(w32.at[:, :, e, j, :], wqkv.at[m * NPAIR + j, :, e],
                                  sem_w.at[m * NPAIR + j]).start()

    def wait_item(i):
        pltpu.make_async_copy(wqkv.at[i], wqkv.at[i], sem_w.at[i]).wait()

    for r in range(8):
        ax_copy(r).start()
    xz_copy = pltpu.make_async_copy(bx_hbm.at[:, pl.ds(SEG - 8, 8), :], xz_raw, sem_xz.at[0])
    xz_copy.start()
    for j in range(FIRST_ITEMS + 2):
        start_pair(0, j)
    for cp in f_copies:
        cp.start()

    _build_dft_matrices(m1, m2)
    m1, m2 = m1.bitcast(i32), m2.bitcast(i32)

    def wait_x(r):
        for i in {0: (0,), 1: (1, 2), 3: (3, 4, 5), 6: (6, 7)}.get(r, ()):
            ax_copy(i).wait()
        if r == 6:
            xz_copy.wait()
            for i in range(2):
                wait_item(i)

    def prepare_early():
        interleave = _interleave_heads(wqkv, (0, 1), 16)
        for c in range(0, NSEG, 4):
            xz[c * 8:(c + 4) * 8, :] = xz_raw[c:c + 4].astype(f32).reshape(32, D)
            next(interleave)
            yield

    _forward(xv, m1, m2, gbuf, wait_x, prepare_early())

    for j in range(FIRST_ITEMS + 2, NPAIR):
        start_pair(0, j)
    for j in range(8):
        start_pair(1, j)

    def filter_groups(t):
        for k1 in range(8):
            extract = (_lo_f32, _hi_f32)[k1 % 2]
            g = t + (16 * k1 if k1 < 4 else 16 * ((8 - k1) % 4) + 8)
            yield from _filter_rows(g, gbuf, lambda k: tuple(
                extract(w[k, pl.ds(32 * t + k1 // 2, 8, stride=4), :]) for w in (wrv, wiv)))

    def project_early(items, interleave_work, filter_work=iter(()), pieces=lambda n: 0):
        for n, (i, e, r0) in enumerate((i, e, r0) for i in items for e in range(2)
                                       for r0 in range(0, NSEG * 8, 64)):
            res = _dot(xz[r0:r0 + 64, :], _head_weight(wqkv, i, e))
            early_rows[2 * i + e, r0:r0 + 64, :] = res
            gbuf[65 + i % 2, 0, :, 0:128] = res[56:64]
            next(interleave_work, None)
            for _ in range(pieces(n)):
                next(filter_work, None)

    @pl.loop(0, FIRST_ITEMS)
    def _(i):
        wait_item(i + 2)
        filter_work = (x for n in range(13) for x in _filter_rows(13 * i + n, gbuf))
        project_early((i,), _interleave_heads(wqkv, (i + 2,), 16),
                      filter_work, lambda n: 4 if n % 2 == 0 else 3)

    for j in range(8, NPAIR):
        start_pair(1, j)
    for cp in f_copies:
        cp.wait()

    @pl.loop(0, 4)
    def _(u):
        for i in range(4):
            start_pair(2, 4 * u + i)

        @pl.loop(2 * u, 2 * u + 2)
        def _(t):
            ahead = (FIRST_ITEMS + 2 * t + 2, FIRST_ITEMS + 2 * t + 3)
            for i in ahead:
                wait_item(i)
            project_early((FIRST_ITEMS + 2 * t, FIRST_ITEMS + 2 * t + 1),
                          _interleave_heads(wqkv, ahead, 32),
                          filter_groups(t), lambda n: 3 if n % 8 == 0 else 2)

    bx_copy(0).start()
    for cp in wo_copies:
        cp.start()
    list(_filter_rows(64, gbuf, lambda k: tuple(
        jnp.broadcast_to(w[:, k * 128:(k + 1) * 128].astype(f32), (8, 128)) for w in (wnr, wni))))

    done = FIRST_ITEMS + 16
    for i in range(done + 2, 2 * NPAIR):
        wait_item(i)
    _inverse(m1, m2, gbuf, rbuf, yv, _interleave_heads(wqkv, range(done + 2, 2 * NPAIR), 32))

    steps = (EARLY_ITEMS - done) // 2
    per_step = NPAIR // steps
    assert done + 2 * steps == EARLY_ITEMS and per_step * steps == NPAIR
    for i in range(2 * NPAIR, 3 * NPAIR):
        wait_item(i)

    @pl.loop(0, steps)
    def _(t):
        ahead = [2 * NPAIR + per_step * t + i for i in range(per_step)]
        project_early((done + 2 * t, done + 2 * t + 1), _interleave_heads(wqkv, ahead, 32))

    for cp in wo_copies:
        cp.wait()
    for c in range(1, NCHUNK):
        bx_copy(c).start()
    for r in range(8):
        ya_copy(r).start()
    h_ref[0:M, :] = mem0_ref[...].astype(f32)
    wo32 = wo.bitcast(i32)

    @pl.loop(0, NCHUNK)
    def _(c):
        bx_copy(c).wait()
        for i in range(SCHUNK):
            _segment(c * SCHUNK + i, wqkv, wo32, xs, early_rows, h_ref, outs)
        yb_copy(c).start()

    for r in range(8):
        ya_copy(r).wait()
    for c in range(NCHUNK):
        yb_copy(c).wait()


@functools.partial(jax.jit, static_argnames=("B_seg_len",))
def pallas_concat_heads__spectral_gfnet__memory_aug_recurrent_mem_tr__prompt_kernel(
    A_x, A_w_r, A_w_i, B_x, B_mem0, B_Wq, B_Wk, B_Wv, B_Wo, B_seg_len,
):
    assert A_x.shape == (1, S, D) and B_x.shape == (1, S, D) and B_mem0.shape == (1, M, D)
    assert A_w_r.shape == (S, D // 2 + 1) and B_Wq.shape == (D, H, DH) and B_Wo.shape == (H, DH, D)
    assert B_seg_len == SEG
    hbm = pl.BlockSpec(memory_space=pl.ANY)
    out = pl.pallas_call(
        _kernel,
        out_shape=jax.ShapeDtypeStruct((S // 16, 16, 2 * D), bf16),
        in_specs=[hbm] * 9,
        out_specs=hbm,
        scratch_shapes=[
            pltpu.VMEM((8, 128, D), i32),
            pltpu.VMEM((16, D // 4 + 8, 128), i32),
            pltpu.VMEM((16, D // 4 + 8, 128), i32),
            pltpu.VMEM((1, S), bf16),
            pltpu.VMEM((1, S), bf16),
            pltpu.VMEM((4, 3, 128, 128), bf16),
            pltpu.VMEM((16, 3, 128, 128), bf16),
            pltpu.VMEM((67, 16, 8, 256), f32),
            pltpu.VMEM((4, 4, 2, 128, 128), f32),
            pltpu.VMEM((8, 128, D), i32),
            pltpu.VMEM((3 * NPAIR, D // 16, 2, 8, DH), i32),
            pltpu.VMEM((8, H * DH, 128), bf16),
            pltpu.VMEM((NSEG, SEG, D), bf16),
            pltpu.VMEM((NSEG, 8, D), bf16),
            pltpu.VMEM((NSEG * 8, D), f32),
            pltpu.VMEM((2 * EARLY_ITEMS, NSEG * 8, DH), f32),
            pltpu.VMEM((M, D), bf16),
            pltpu.VMEM((L, D), f32),
            pltpu.VMEM((S // 16, 16, D), bf16),
            pltpu.SemaphoreType.DMA((8,)),
            pltpu.SemaphoreType.DMA((1,)),
            pltpu.SemaphoreType.DMA((3 * NPAIR,)),
            pltpu.SemaphoreType.DMA((1,)),
            pltpu.SemaphoreType.DMA((NCHUNK,)),
            pltpu.SemaphoreType.DMA((1,)),
            pltpu.SemaphoreType.DMA((1,)),
            pltpu.SemaphoreType.DMA((1,)),
        ],
        compiler_params=pltpu.CompilerParams(vmem_limit_bytes=100 * 1024 * 1024),
    )(
        A_x.reshape(S // 16, 16, D), A_w_r.T, A_w_i.T,
        B_x.reshape(NSEG, SEG, D), B_mem0.reshape(M, D),
        B_Wq.reshape(D // 16, 8, 2, H, DH), B_Wk.reshape(D // 16, 8, 2, H, DH),
        B_Wv.reshape(D // 16, 8, 2, H, DH), B_Wo.reshape(H * DH, D),
    )
    return out.reshape(1, S, 2 * D)
```

```python
import functools
import math

import jax
import jax.numpy as jnp
from jax import lax
import jax.experimental.pallas as pl
import jax.experimental.pallas.tpu as pltpu

bf16, f32, i32 = jnp.bfloat16, jnp.float32, jnp.int32

S, D = 2048, 1024
H, DH = 32, 128
M, SEG = 8, 32
L = M + SEG
NSEG = S // SEG
NPAIR = H // 2
FIRST_ITEMS = 5
EARLY_ITEMS = 25
SCHUNK = 2
NCHUNK = NSEG // SCHUNK

_NN = (((1,), (0,)), ((), ()))
_NT = (((1,), (1,)), ((), ()))
_HI16 = -65536
_R2 = math.sqrt(0.5)
_SCALE = 2.0 ** -5


def _dot(a, b, dims=_NN):
    return lax.dot_general(a, b, dims, preferred_element_type=f32)


def _lo_f32(w):
    return pltpu.bitcast(w << 16, f32)


def _hi_f32(w):
    return pltpu.bitcast(w & _HI16, f32)


def _cadd(a, b):
    return a[0] + b[0], a[1] + b[1]


def _csub(a, b):
    return a[0] - b[0], a[1] - b[1]


def _fft4(x0, x1, x2, x3, sign):
    a, b = _cadd(x0, x2), _csub(x0, x2)
    c, d = _cadd(x1, x3), _csub(x1, x3)
    minus_i = (b[0] + d[1], b[1] - d[0])
    plus_i = (b[0] - d[1], b[1] + d[0])
    if sign < 0:
        return _cadd(a, c), minus_i, _csub(a, c), plus_i
    return _cadd(a, c), plus_i, _csub(a, c), minus_i


def _twiddle16(x, m, sign):
    if m == 0:
        return x
    if m == 4:
        return (-x[1], x[0]) if sign > 0 else (x[1], -x[0])
    if m == 2:
        if sign > 0:
            return (x[0] - x[1]) * _R2, (x[0] + x[1]) * _R2
        return (x[0] + x[1]) * _R2, (x[1] - x[0]) * _R2
    if m == 6:
        if sign > 0:
            return (x[0] + x[1]) * -_R2, (x[0] - x[1]) * _R2
        return (x[1] - x[0]) * _R2, (x[0] + x[1]) * -_R2
    c, s = math.cos(2 * math.pi * m / 16), sign * math.sin(2 * math.pi * m / 16)
    return x[0] * c - x[1] * s, x[0] * s + x[1] * c


def _rfft8(x):
    s04, d04 = x[0] + x[4], x[0] - x[4]
    s26, d26 = x[2] + x[6], x[2] - x[6]
    s15, d15 = x[1] + x[5], x[1] - x[5]
    s37, d37 = x[3] + x[7], x[3] - x[7]
    e, o = s04 + s26, s15 + s37
    p, q = (d15 - d37) * _R2, (d15 + d37) * _R2
    return (e + o, e - o), (d04 + p, -(d26 + q)), (s04 - s26, s37 - s15), (d04 - p, d26 - q)


def _irfft8(r0, r1, r2, r3):
    a0, a4 = r0[0] + r0[1], r0[0] - r0[1]
    e0, e2 = a0 + r2[0], a0 - r2[0]
    e1, e3 = a4 - r2[1], a4 + r2[1]
    o0, o2 = r1[0] + r3[0], r3[1] - r1[1]
    dr, si = r1[0] - r3[0], r1[1] + r3[1]
    o1, o3 = (dr - si) * _R2, (dr + si) * -_R2
    return [e0 + o0, e1 + o1, e2 + o2, e3 + o3, e0 - o0, e1 - o1, e2 - o2, e3 - o3]


def _halves(w):
    return pltpu.bitcast(w, bf16)


def _complex_product(apply, m, xr, xi, xs, conjugate):
    shared = apply(_halves(m[0]), xs)
    for_re, for_im = (2, 1) if conjugate else (1, 2)
    return apply(_halves(m[for_re]), xi) + shared, apply(_halves(m[for_im]), xr) + shared


def _from_left(m, x):
    return _dot(m, x, _NT)


def _from_right(m, x):
    return _dot(x, m)


def _build_dft_matrices(m1, m2):
    ri = lax.broadcasted_iota(i32, (128, 128), 0)
    ci = lax.broadcasted_iota(i32, (128, 128), 1)
    ang = ((ri * ci) & 127).astype(f32) * (2 * math.pi / 128)
    cb, sb = jnp.cos(ang), jnp.sin(ang)
    ang = (ri[0:16] * ci[0:16]).astype(f32) * (2 * math.pi / S)
    ct_all, st_all = jnp.cos(ang) * _SCALE, jnp.sin(ang) * _SCALE

    def rotated(rows, a):
        ct, st = ct_all[a:a + 1], st_all[a:a + 1]
        return cb[0:rows] * ct - sb[0:rows] * st, sb[0:rows] * ct + cb[0:rows] * st

    def store(m, c, s):
        m[0], m[1], m[2] = c.astype(bf16), (-(c + s)).astype(bf16), (s - c).astype(bf16)

    for p in range(4):
        c0, s0 = rotated(64, 2 * p)
        c1, s1 = rotated(64, 2 * (4 if p == 0 else 8 - p))
        if p == 0:
            nyquist = jnp.where((ci[0:64] & 1) == 0, _SCALE, -_SCALE)
            s0 = jnp.where(ri[0:64] == 0, nyquist, -s0)
            m1[0, 0] = jnp.concatenate([c0, s0], axis=0).astype(bf16)
            m1[0, 1] = jnp.concatenate([c1, -s1], axis=0).astype(bf16)
        else:
            store(m1.at[p], jnp.concatenate([c0, c1], axis=0), jnp.concatenate([s0, -s1], axis=0))

    for a in range(16):
        store(m2.at[a], *rotated(128, a))


def _forward(xv, m1, m2, gbuf, wait_x, late_work):
    sub = lax.broadcasted_iota(i32, (8, 128), 0)
    inputs = {}

    def butterflies(a, quarter):
        extract = (_lo_f32, _hi_f32)[a % 2]
        for g in range(2 * quarter, 2 * quarter + 2):
            u = _rfft8([extract(xv[a // 2, g * 16:(g + 1) * 16, j * 128:(j + 1) * 128])
                        for j in range(8)])
            for p in range(4):
                parts = u[p] if p == 0 else (*u[p], u[p][0] + u[p][1])
                for k, part in enumerate(parts):
                    inputs.setdefault((a, p, k), []).append(part)

    def feature_stage(a, p):
        u = [jnp.concatenate(inputs.pop((a, p, k)), axis=0).astype(bf16)
             for k in range(3 if p else 2)]
        if p > 0:
            tr, ti = _complex_product(_from_left, m1.at[p], *u, True)
            return tr, jnp.concatenate([ti[0:64], -ti[64:128]], axis=0)
        t0, t1 = [_from_left(_halves(m1[0, k]), u[k]) for k in range(2)]
        tr = [jnp.where(sub == 0, t0[0:8] * 0.5, t0[0:8]), t0[8:64], t1[0:64],
              jnp.where(sub == 0, t0[64:72] * 0.5, 0.0)]
        ti = [jnp.where(sub == 0, 0.0, t0[64:72]), t0[72:128], t1[64:128],
              jnp.zeros((8, 128), f32)]
        return jnp.concatenate(tr, axis=0), jnp.concatenate(ti, axis=0)

    def sequence_stage(a, p, t):
        for k, g in enumerate(_complex_product(_from_right, m2.at[a], *t, t[0] + t[1], True)):
            for blk in range(16):
                gbuf[p * 16 + blk, a, :, k * 128:(k + 1) * 128] = g[blk * 8:(blk + 1) * 8]
            if p == 0:
                gbuf[64, a, :, k * 128:(k + 1) * 128] = g[128:136]

    wait_x(0)
    for quarter in range(4):
        butterflies(0, quarter)
    pending = None
    for i in range(64):
        a, p = divmod(i, 4)
        t = feature_stage(a, p)
        if a < 15:
            if p == 0 and a % 2 == 1:
                wait_x((a + 1) // 2)
            butterflies(a + 1, p)
        if i >= 44:
            next(late_work, None)
        if pending is not None:
            sequence_stage(*pending)
        pending = (a, p, t)
    sequence_stage(*pending)


def _filter_rows(g, gbuf, filt=None):
    def load(slots):
        return [(gbuf[g, a, :, 0:128], gbuf[g, a, :, 128:256]) for a in slots]

    def store(slots, values):
        for a, (re, im) in zip(slots, values):
            gbuf[g, a, :, 0:128] = re
            gbuf[g, a, :, 128:256] = im

    if filt is None:
        for a0 in range(4):
            slots = range(a0, 16, 4)
            ys = _fft4(*load(slots), -1)
            store(slots, [_twiddle16(ys[k0], a0 * k0, -1) for k0 in range(4)])
            yield
        return
    for k0 in range(4):
        slots = range(4 * k0, 4 * k0 + 4)
        ys = []
        for k1, (xr, xi) in enumerate(_fft4(*load(slots), -1)):
            wr, wi = filt(k0 + 4 * k1)
            ys.append((xr * wr - xi * wi, xr * wi + xi * wr))
        ys = _fft4(*ys, +1)
        store(slots, [_twiddle16(ys[a0], a0 * k0, +1) for a0 in range(4)])
        yield
    for a0 in range(4):
        slots = range(a0, 16, 4)
        store(slots, _fft4(*load(slots), +1))
        yield


def _inverse(m1, m2, gbuf, rbuf, yv):
    sub = lax.broadcasted_iota(i32, (8, 128), 0)
    sign = jnp.where(lax.broadcasted_iota(i32, (128, 128), 1) < 64, 1.0, -1.0)

    def sequence_stage(a, p):
        hr, hi = [gbuf[p * 16:(p + 1) * 16, a, :, k * 128:(k + 1) * 128].reshape(128, 128)
                  for k in range(2)]
        if p > 0:
            zr, zi = _complex_product(_from_left, m2.at[a], hr.astype(bf16), hi.astype(bf16),
                                      (hr + hi).astype(bf16), False)
            return zr, zi * sign
        nr, ni = gbuf[64, a, :, 0:128], gbuf[64, a, :, 128:256]
        low = ([hr[0:64], jnp.where(sub == 0, nr, hi[0:8]), hi[8:64]],
               [hi[0:64], jnp.where(sub == 0, ni, -hr[0:8]), -hr[8:64]])
        high = ([hr[64:128], hi[64:128]], [hi[64:128], -hr[64:128]])
        zs = []
        for re, im in (low, high):
            re, im = jnp.concatenate(re, axis=0), jnp.concatenate(im, axis=0)
            zs.append(_from_left(_halves(m2[a, 1]), im.astype(bf16))
                      + _from_left(_halves(m2[a, 0]), (re + im).astype(bf16)))
        return zs

    def feature_stage(a, p, z):
        if p > 0:
            v = _complex_product(_from_right, m1.at[p], *z, z[0] + z[1], False)
        else:
            v = [_from_right(_halves(m1[0, k]), z[k]) for k in range(2)]
        rbuf[a % 4, p, 0] = v[0]
        rbuf[a % 4, p, 1] = v[1]

    def butterflies(r, eighth):
        for g in range(2 * eighth, 2 * eighth + 2):
            rows = slice(g * 8, (g + 1) * 8)
            ys = [_irfft8(*[(rbuf[a % 4, p, 0, rows, :], rbuf[a % 4, p, 1, rows, :])
                            for p in range(4)]) for a in (2 * r, 2 * r + 1)]
            for j in range(8):
                even = pltpu.bitcast(ys[0][j].astype(bf16).astype(f32), i32)
                odd = pltpu.bitcast(ys[1][j].astype(bf16).astype(f32), i32)
                yv[r, rows, j * 128:(j + 1) * 128] = lax.shift_right_logical(even, 16) | odd

    pending = {}
    for i in range(64 + 9):
        if i < 64:
            pending[i] = sequence_stage(*divmod(i, 4))
        if 1 <= i <= 64:
            feature_stage(*divmod(i - 1, 4), pending.pop(i - 1))
        if i >= 9:
            butterflies(*divmod(i - 9, 8))


def _interleave_heads(w, items, pieces=1):
    per_piece = D // 16 // pieces
    for first in range(0, D // 16, per_piece):
        for i in items:
            for c in range(first, first + per_piece, 2):
                even, odd = w[i, c:c + 2, 0], w[i, c:c + 2, 1]
                w[i, c:c + 2, 0] = (even & 0xFFFF) | (odd << 16)
                w[i, c:c + 2, 1] = lax.shift_right_logical(even, 16) | (odd & _HI16)
        yield


def _head_weight(w, i, e):
    return _halves(w[i, :, e].reshape(D // 2, DH))


def _segment(s, wqkv, wo32, xs, early_rows, h_ref, outs):
    z0 = pl.multiple_of(s * 8, 8)
    h_ref[M:L, :] = xs[s].astype(f32)
    row = lax.broadcasted_iota(i32, (L, L), 0)
    col = lax.broadcasted_iota(i32, (L, L), 1)
    mask = (row < M) | (row >= col)

    def project(h):
        items = [m * NPAIR + h // 2 for m in range(3)]
        ws = [_head_weight(wqkv, i, h % 2) for i in items]
        rows = [L - 8 if i < EARLY_ITEMS else L for i in items]
        if h == 0:
            first = [_dot(h_ref[0:n, 0:D // 2], w[0:D // 2]) for n, w in zip(rows, ws)]
            qkv = [_dot(h_ref[0:n, D // 2:D], w[D // 2:D]) + f for n, w, f in zip(rows, ws, first)]
        else:
            qkv = [_dot(h_ref[0:n, :], w) for n, w in zip(rows, ws)]
        return [jnp.concatenate([v, early_rows[2 * i + h % 2, pl.ds(z0, 8), :]], axis=0)
                if i < EARLY_ITEMS else v for v, i in zip(qkv, items)]

    def probabilities(q, k):
        sc = _dot(q, k.astype(bf16), _NT) * DH ** -0.5
        sc = jnp.where(mask, sc, -1e9)
        e = jnp.exp(sc - jnp.max(sc, axis=-1, keepdims=True))
        return e * pltpu.reciprocal(jnp.sum(e, axis=-1, keepdims=True), approx=False)

    def out_proj(o, n, lo, hi):
        w = _halves(wo32[n, lo * DH // 2:hi * DH // 2, :])
        return _dot(jnp.concatenate(o[lo:hi], axis=1), w)

    lag_scores, lag_mix, split = 2, 4, 24
    state, o, part = {}, [None] * H, [None] * 8
    for t in range(H + 8):
        if t < H:
            state[t] = project(t)
        else:
            part[t - H] = out_proj(o, t - H, 0, split)
        if 0 <= t - lag_scores < H:
            q, k, v = state[t - lag_scores]
            state[t - lag_scores] = (probabilities(q, k), v)
        if 0 <= t - lag_mix < H:
            p, v = state.pop(t - lag_mix)
            o[t - lag_mix] = _dot(p, v.astype(bf16))
    for n in range(8):
        res = out_proj(o, n, split, H) + part[n]
        h_ref[0:M, n * 128:(n + 1) * 128] = res[0:M]
        for i in range(SEG // 16):
            outs[2 * s + i, :, n * 128:(n + 1) * 128] = res[M + 16 * i:M + 16 * i + 16].astype(bf16)


def _kernel(ax_hbm, wr_hbm, wi_hbm, bx_hbm, mem0_hbm, wq_hbm, wk_hbm, wv_hbm, wo_hbm, out_hbm,
            xv, wrv, wiv, wnr, wni, m1, m2, gbuf, rbuf, yv,
            wqkv, wo, xs, xz_raw, xz, early_rows, mem0_ref, h_ref, outs,
            sem_ax, sem_f, sem_w, sem_wo, sem_bx, sem_xz, sem_ya, sem_yb):
    ax32 = ax_hbm.bitcast(i32)
    out32 = out_hbm.bitcast(i32)

    def ax_copy(r):
        return pltpu.make_async_copy(ax32.at[:, r, :], xv.at[r], sem_ax.at[r])

    def ya_copy(r):
        return pltpu.make_async_copy(yv.at[r], out32.at[:, r, pl.ds(0, D)], sem_ya.at[0])

    def bx_copy(c):
        return pltpu.make_async_copy(bx_hbm.at[pl.ds(c * SCHUNK, SCHUNK)],
                                     xs.at[pl.ds(c * SCHUNK, SCHUNK)], sem_bx.at[c])

    def yb_copy(c):
        rows = pl.ds(c * (SCHUNK * SEG // 16), SCHUNK * SEG // 16)
        return pltpu.make_async_copy(outs.at[rows], out_hbm.at[rows, :, pl.ds(D, D)], sem_yb.at[0])

    f_copies = [pltpu.make_async_copy(src.at[pl.ds(0, D // 2), pl.ds(k1 * 128, 128)],
                                      dst.at[k1, pl.ds(0, D // 4)].bitcast(bf16), sem_f.at[0])
                for k1 in range(16) for src, dst in ((wr_hbm, wrv), (wi_hbm, wiv))]
    f_copies += [pltpu.make_async_copy(src.at[pl.ds(D // 2, 1), :], dst, sem_f.at[0])
                 for src, dst in ((wr_hbm, wnr), (wi_hbm, wni))]
    wo_copies = [pltpu.make_async_copy(wo_hbm.at[:, pl.ds(n * 128, 128)], wo.at[n], sem_wo.at[0])
                 for n in range(8)]
    wo_copies.append(pltpu.make_async_copy(mem0_hbm, mem0_ref, sem_wo.at[0]))

    def start_pair(m, j):
        w32 = (wq_hbm, wk_hbm, wv_hbm)[m].bitcast(i32)
        for e in range(2):
            pltpu.make_async_copy(w32.at[:, :, e, j, :], wqkv.at[m * NPAIR + j, :, e],
                                  sem_w.at[m * NPAIR + j]).start()

    def wait_item(i):
        pltpu.make_async_copy(wqkv.at[i], wqkv.at[i], sem_w.at[i]).wait()

    for r in range(8):
        ax_copy(r).start()
    xz_copy = pltpu.make_async_copy(bx_hbm.at[:, pl.ds(SEG - 8, 8), :], xz_raw, sem_xz.at[0])
    xz_copy.start()
    for j in range(FIRST_ITEMS + 2):
        start_pair(0, j)
    for cp in f_copies:
        cp.start()

    _build_dft_matrices(m1, m2)
    m1, m2 = m1.bitcast(i32), m2.bitcast(i32)

    def wait_x(r):
        for i in {0: (0,), 1: (1, 2), 3: (3, 4, 5), 6: (6, 7)}.get(r, ()):
            ax_copy(i).wait()
        if r == 6:
            xz_copy.wait()
            for i in range(2):
                wait_item(i)

    def prepare_early():
        interleave = _interleave_heads(wqkv, (0, 1), 16)
        for c in range(0, NSEG, 4):
            xz[c * 8:(c + 4) * 8, :] = xz_raw[c:c + 4].astype(f32).reshape(32, D)
            next(interleave)
            yield

    _forward(xv, m1, m2, gbuf, wait_x, prepare_early())

    for j in range(FIRST_ITEMS + 2, NPAIR):
        start_pair(0, j)
    for j in range(8):
        start_pair(1, j)

    def filter_groups(t):
        for k1 in range(8):
            extract = (_lo_f32, _hi_f32)[k1 % 2]
            g = t + (16 * k1 if k1 < 4 else 16 * ((8 - k1) % 4) + 8)
            yield from _filter_rows(g, gbuf, lambda k: tuple(
                extract(w[k, pl.ds(32 * t + k1 // 2, 8, stride=4), :]) for w in (wrv, wiv)))

    def project_early(items, interleave_work, filter_work=iter(()), pieces=lambda n: 0):
        for n, (i, e, r0) in enumerate((i, e, r0) for i in items for e in range(2)
                                       for r0 in range(0, NSEG * 8, 64)):
            res = _dot(xz[r0:r0 + 64, :], _head_weight(wqkv, i, e))
            early_rows[2 * i + e, r0:r0 + 64, :] = res
            gbuf[65 + i % 2, 0, :, 0:128] = res[56:64]
            next(interleave_work, None)
            for _ in range(pieces(n)):
                next(filter_work, None)

    @pl.loop(0, FIRST_ITEMS)
    def _(i):
        wait_item(i + 2)
        filter_work = (x for n in range(13) for x in _filter_rows(13 * i + n, gbuf))
        project_early((i,), _interleave_heads(wqkv, (i + 2,), 16),
                      filter_work, lambda n: 4 if n % 2 == 0 else 3)

    for j in range(8, NPAIR):
        start_pair(1, j)
    for cp in f_copies:
        cp.wait()

    @pl.loop(0, 4)
    def _(u):
        for i in range(4):
            start_pair(2, 4 * u + i)

        @pl.loop(2 * u, 2 * u + 2)
        def _(t):
            ahead = (FIRST_ITEMS + 2 * t + 2, FIRST_ITEMS + 2 * t + 3)
            for i in ahead:
                wait_item(i)
            project_early((FIRST_ITEMS + 2 * t, FIRST_ITEMS + 2 * t + 1),
                          _interleave_heads(wqkv, ahead, 32),
                          filter_groups(t), lambda n: 3 if n % 8 == 0 else 2)

    bx_copy(0).start()
    for cp in wo_copies:
        cp.start()
    list(_filter_rows(64, gbuf, lambda k: tuple(
        jnp.broadcast_to(w[:, k * 128:(k + 1) * 128].astype(f32), (8, 128)) for w in (wnr, wni))))

    done = FIRST_ITEMS + 16
    wait_item(done + 2)
    list(_interleave_heads(wqkv, (done + 2,)))
    _inverse(m1, m2, gbuf, rbuf, yv)

    steps = (EARLY_ITEMS - done) // 2
    per_step = (3 * NPAIR - done - 3) // steps
    assert done + 2 * steps == EARLY_ITEMS and done + 3 + per_step * steps == 3 * NPAIR
    for i in range(done + 3, 3 * NPAIR):
        wait_item(i)

    @pl.loop(0, steps)
    def _(t):
        ahead = [done + 3 + per_step * t + i for i in range(per_step)]
        project_early((done + 2 * t, done + 2 * t + 1), _interleave_heads(wqkv, ahead, 32))

    for cp in wo_copies:
        cp.wait()
    for c in range(1, NCHUNK):
        bx_copy(c).start()
    for r in range(8):
        ya_copy(r).start()
    h_ref[0:M, :] = mem0_ref[...].astype(f32)
    wo32 = wo.bitcast(i32)

    @pl.loop(0, NCHUNK)
    def _(c):
        bx_copy(c).wait()
        for i in range(SCHUNK):
            _segment(c * SCHUNK + i, wqkv, wo32, xs, early_rows, h_ref, outs)
        yb_copy(c).start()

    for r in range(8):
        ya_copy(r).wait()
    for c in range(NCHUNK):
        yb_copy(c).wait()


@functools.partial(jax.jit, static_argnames=("B_seg_len",))
def pallas_concat_heads__spectral_gfnet__memory_aug_recurrent_mem_tr__prompt_kernel(
    A_x, A_w_r, A_w_i, B_x, B_mem0, B_Wq, B_Wk, B_Wv, B_Wo, B_seg_len,
):
    assert A_x.shape == (1, S, D) and B_x.shape == (1, S, D) and B_mem0.shape == (1, M, D)
    assert A_w_r.shape == (S, D // 2 + 1) and B_Wq.shape == (D, H, DH) and B_Wo.shape == (H, DH, D)
    assert B_seg_len == SEG
    hbm = pl.BlockSpec(memory_space=pl.ANY)
    out = pl.pallas_call(
        _kernel,
        out_shape=jax.ShapeDtypeStruct((S // 16, 16, 2 * D), bf16),
        in_specs=[hbm] * 9,
        out_specs=hbm,
        scratch_shapes=[
            pltpu.VMEM((8, 128, D), i32),
            pltpu.VMEM((16, D // 4 + 8, 128), i32),
            pltpu.VMEM((16, D // 4 + 8, 128), i32),
            pltpu.VMEM((1, S), bf16),
            pltpu.VMEM((1, S), bf16),
            pltpu.VMEM((4, 3, 128, 128), bf16),
            pltpu.VMEM((16, 3, 128, 128), bf16),
            pltpu.VMEM((67, 16, 8, 256), f32),
            pltpu.VMEM((4, 4, 2, 128, 128), f32),
            pltpu.VMEM((8, 128, D), i32),
            pltpu.VMEM((3 * NPAIR, D // 16, 2, 8, DH), i32),
            pltpu.VMEM((8, H * DH, 128), bf16),
            pltpu.VMEM((NSEG, SEG, D), bf16),
            pltpu.VMEM((NSEG, 8, D), bf16),
            pltpu.VMEM((NSEG * 8, D), f32),
            pltpu.VMEM((2 * EARLY_ITEMS, NSEG * 8, DH), f32),
            pltpu.VMEM((M, D), bf16),
            pltpu.VMEM((L, D), f32),
            pltpu.VMEM((S // 16, 16, D), bf16),
            pltpu.SemaphoreType.DMA((8,)),
            pltpu.SemaphoreType.DMA((1,)),
            pltpu.SemaphoreType.DMA((3 * NPAIR,)),
            pltpu.SemaphoreType.DMA((1,)),
            pltpu.SemaphoreType.DMA((NCHUNK,)),
            pltpu.SemaphoreType.DMA((1,)),
            pltpu.SemaphoreType.DMA((1,)),
            pltpu.SemaphoreType.DMA((1,)),
        ],
        compiler_params=pltpu.CompilerParams(vmem_limit_bytes=100 * 1024 * 1024),
    )(
        A_x.reshape(S // 16, 16, D), A_w_r.T, A_w_i.T,
        B_x.reshape(NSEG, SEG, D), B_mem0.reshape(M, D),
        B_Wq.reshape(D // 16, 8, 2, H, DH), B_Wk.reshape(D // 16, 8, 2, H, DH),
        B_Wv.reshape(D // 16, 8, 2, H, DH), B_Wo.reshape(H * DH, D),
    )
    return out.reshape(1, S, 2 * D)
```

```python
import functools
import math

import jax
import jax.numpy as jnp
from jax import lax
import jax.experimental.pallas as pl
import jax.experimental.pallas.tpu as pltpu

bf16, f32, i32 = jnp.bfloat16, jnp.float32, jnp.int32

S, D = 2048, 1024
H, DH = 32, 128
M, SEG = 8, 32
L = M + SEG
NSEG = S // SEG
NPAIR = H // 2
FIRST_ITEMS = 6
EARLY_ITEMS = 26
SCHUNK = 2
NCHUNK = NSEG // SCHUNK

_NN = (((1,), (0,)), ((), ()))
_NT = (((1,), (1,)), ((), ()))
_HI16 = -65536
_R2 = math.sqrt(0.5)
_SCALE = 2.0 ** -5


def _dot(a, b, dims=_NN):
    return lax.dot_general(a, b, dims, preferred_element_type=f32)


def _lo_f32(w):
    return pltpu.bitcast(w << 16, f32)


def _hi_f32(w):
    return pltpu.bitcast(w & _HI16, f32)


def _cadd(a, b):
    return a[0] + b[0], a[1] + b[1]


def _csub(a, b):
    return a[0] - b[0], a[1] - b[1]


def _fft4(x0, x1, x2, x3, sign):
    a, b = _cadd(x0, x2), _csub(x0, x2)
    c, d = _cadd(x1, x3), _csub(x1, x3)
    minus_i = (b[0] + d[1], b[1] - d[0])
    plus_i = (b[0] - d[1], b[1] + d[0])
    if sign < 0:
        return _cadd(a, c), minus_i, _csub(a, c), plus_i
    return _cadd(a, c), plus_i, _csub(a, c), minus_i


def _twiddle16(x, m, sign):
    if m == 0:
        return x
    if m == 4:
        return (-x[1], x[0]) if sign > 0 else (x[1], -x[0])
    if m == 2:
        if sign > 0:
            return (x[0] - x[1]) * _R2, (x[0] + x[1]) * _R2
        return (x[0] + x[1]) * _R2, (x[1] - x[0]) * _R2
    if m == 6:
        if sign > 0:
            return (x[0] + x[1]) * -_R2, (x[0] - x[1]) * _R2
        return (x[1] - x[0]) * _R2, (x[0] + x[1]) * -_R2
    c, s = math.cos(2 * math.pi * m / 16), sign * math.sin(2 * math.pi * m / 16)
    return x[0] * c - x[1] * s, x[0] * s + x[1] * c


def _rfft8(x):
    s04, d04 = x[0] + x[4], x[0] - x[4]
    s26, d26 = x[2] + x[6], x[2] - x[6]
    s15, d15 = x[1] + x[5], x[1] - x[5]
    s37, d37 = x[3] + x[7], x[3] - x[7]
    e, o = s04 + s26, s15 + s37
    p, q = (d15 - d37) * _R2, (d15 + d37) * _R2
    return (e + o, e - o), (d04 + p, -(d26 + q)), (s04 - s26, s37 - s15), (d04 - p, d26 - q)


def _irfft8(r0, r1, r2, r3):
    a0, a4 = r0[0] + r0[1], r0[0] - r0[1]
    e0, e2 = a0 + r2[0], a0 - r2[0]
    e1, e3 = a4 - r2[1], a4 + r2[1]
    o0, o2 = r1[0] + r3[0], r3[1] - r1[1]
    dr, si = r1[0] - r3[0], r1[1] + r3[1]
    o1, o3 = (dr - si) * _R2, (dr + si) * -_R2
    return [e0 + o0, e1 + o1, e2 + o2, e3 + o3, e0 - o0, e1 - o1, e2 - o2, e3 - o3]


def _halves(w):
    return pltpu.bitcast(w, bf16)


def _complex_product(apply, m, xr, xi, xs, conjugate):
    shared = apply(_halves(m[0]), xs)
    for_re, for_im = (2, 1) if conjugate else (1, 2)
    return apply(_halves(m[for_re]), xi) + shared, apply(_halves(m[for_im]), xr) + shared


def _from_left(m, x):
    return _dot(m, x, _NT)


def _from_right(m, x):
    return _dot(x, m)


def _build_dft_matrices(m1, m2):
    ri = lax.broadcasted_iota(i32, (128, 128), 0)
    ci = lax.broadcasted_iota(i32, (128, 128), 1)
    ang = ((ri * ci) & 127).astype(f32) * (2 * math.pi / 128)
    cb, sb = jnp.cos(ang), jnp.sin(ang)
    ang = (ri[0:16] * ci[0:16]).astype(f32) * (2 * math.pi / S)
    ct_all, st_all = jnp.cos(ang) * _SCALE, jnp.sin(ang) * _SCALE

    def rotated(rows, a):
        ct, st = ct_all[a:a + 1], st_all[a:a + 1]
        return cb[0:rows] * ct - sb[0:rows] * st, sb[0:rows] * ct + cb[0:rows] * st

    def store(m, c, s):
        m[0], m[1], m[2] = c.astype(bf16), (-(c + s)).astype(bf16), (s - c).astype(bf16)

    for p in range(4):
        c0, s0 = rotated(64, 2 * p)
        c1, s1 = rotated(64, 2 * (4 if p == 0 else 8 - p))
        if p == 0:
            nyquist = jnp.where((ci[0:64] & 1) == 0, _SCALE, -_SCALE)
            s0 = jnp.where(ri[0:64] == 0, nyquist, -s0)
            m1[0, 0] = jnp.concatenate([c0, s0], axis=0).astype(bf16)
            m1[0, 1] = jnp.concatenate([c1, -s1], axis=0).astype(bf16)
        else:
            store(m1.at[p], jnp.concatenate([c0, c1], axis=0), jnp.concatenate([s0, -s1], axis=0))

    for a in range(16):
        store(m2.at[a], *rotated(128, a))


def _forward(xv, m1, m2, gbuf, wait_x, late_work):
    sub = lax.broadcasted_iota(i32, (8, 128), 0)
    inputs = {}

    def butterflies(a, quarter):
        extract = (_lo_f32, _hi_f32)[a % 2]
        for g in range(2 * quarter, 2 * quarter + 2):
            u = _rfft8([extract(xv[a // 2, g * 16:(g + 1) * 16, j * 128:(j + 1) * 128])
                        for j in range(8)])
            for p in range(4):
                parts = u[p] if p == 0 else (*u[p], u[p][0] + u[p][1])
                for k, part in enumerate(parts):
                    inputs.setdefault((a, p, k), []).append(part)

    def feature_stage(a, p):
        u = [jnp.concatenate(inputs.pop((a, p, k)), axis=0).astype(bf16)
             for k in range(3 if p else 2)]
        if p > 0:
            tr, ti = _complex_product(_from_left, m1.at[p], *u, True)
            return tr, jnp.concatenate([ti[0:64], -ti[64:128]], axis=0)
        t0, t1 = [_from_left(_halves(m1[0, k]), u[k]) for k in range(2)]
        tr = [jnp.where(sub == 0, t0[0:8] * 0.5, t0[0:8]), t0[8:64], t1[0:64],
              jnp.where(sub == 0, t0[64:72] * 0.5, 0.0)]
        ti = [jnp.where(sub == 0, 0.0, t0[64:72]), t0[72:128], t1[64:128],
              jnp.zeros((8, 128), f32)]
        return jnp.concatenate(tr, axis=0), jnp.concatenate(ti, axis=0)

    def sequence_stage(a, p, t):
        for k, g in enumerate(_complex_product(_from_right, m2.at[a], *t, t[0] + t[1], True)):
            for blk in range(16):
                gbuf[p * 16 + blk, a, :, k * 128:(k + 1) * 128] = g[blk * 8:(blk + 1) * 8]
            if p == 0:
                gbuf[64, a, :, k * 128:(k + 1) * 128] = g[128:136]

    wait_x(0)
    for quarter in range(4):
        butterflies(0, quarter)
    pending = None
    for i in range(64):
        a, p = divmod(i, 4)
        t = feature_stage(a, p)
        if a < 15:
            if p == 0 and a % 2 == 1:
                wait_x((a + 1) // 2)
            butterflies(a + 1, p)
        if i >= 44:
            next(late_work, None)
        if pending is not None:
            sequence_stage(*pending)
        pending = (a, p, t)
    sequence_stage(*pending)


def _filter_rows(g, gbuf, filt=None):
    def load(slots):
        return [(gbuf[g, a, :, 0:128], gbuf[g, a, :, 128:256]) for a in slots]

    def store(slots, values):
        for a, (re, im) in zip(slots, values):
            gbuf[g, a, :, 0:128] = re
            gbuf[g, a, :, 128:256] = im

    if filt is None:
        for a0 in range(4):
            slots = range(a0, 16, 4)
            ys = _fft4(*load(slots), -1)
            store(slots, [_twiddle16(ys[k0], a0 * k0, -1) for k0 in range(4)])
            yield
        return
    for k0 in range(4):
        slots = range(4 * k0, 4 * k0 + 4)
        ys = []
        for k1, (xr, xi) in enumerate(_fft4(*load(slots), -1)):
            wr, wi = filt(k0 + 4 * k1)
            ys.append((xr * wr - xi * wi, xr * wi + xi * wr))
        ys = _fft4(*ys, +1)
        store(slots, [_twiddle16(ys[a0], a0 * k0, +1) for a0 in range(4)])
        yield
    for a0 in range(4):
        slots = range(a0, 16, 4)
        store(slots, _fft4(*load(slots), +1))
        yield


def _inverse(m1, m2, gbuf, rbuf, yv):
    sub = lax.broadcasted_iota(i32, (8, 128), 0)
    sign = jnp.where(lax.broadcasted_iota(i32, (128, 128), 1) < 64, 1.0, -1.0)

    def sequence_stage(a, p):
        hr, hi = [gbuf[p * 16:(p + 1) * 16, a, :, k * 128:(k + 1) * 128].reshape(128, 128)
                  for k in range(2)]
        if p > 0:
            zr, zi = _complex_product(_from_left, m2.at[a], hr.astype(bf16), hi.astype(bf16),
                                      (hr + hi).astype(bf16), False)
            return zr, zi * sign
        nr, ni = gbuf[64, a, :, 0:128], gbuf[64, a, :, 128:256]
        low = ([hr[0:64], jnp.where(sub == 0, nr, hi[0:8]), hi[8:64]],
               [hi[0:64], jnp.where(sub == 0, ni, -hr[0:8]), -hr[8:64]])
        high = ([hr[64:128], hi[64:128]], [hi[64:128], -hr[64:128]])
        zs = []
        for re, im in (low, high):
            re, im = jnp.concatenate(re, axis=0), jnp.concatenate(im, axis=0)
            zs.append(_from_left(_halves(m2[a, 1]), im.astype(bf16))
                      + _from_left(_halves(m2[a, 0]), (re + im).astype(bf16)))
        return zs

    def feature_stage(a, p, z):
        if p > 0:
            v = _complex_product(_from_right, m1.at[p], *z, z[0] + z[1], False)
        else:
            v = [_from_right(_halves(m1[0, k]), z[k]) for k in range(2)]
        rbuf[a % 4, p, 0] = v[0]
        rbuf[a % 4, p, 1] = v[1]

    def butterflies(r, eighth):
        for g in range(2 * eighth, 2 * eighth + 2):
            rows = slice(g * 8, (g + 1) * 8)
            ys = [_irfft8(*[(rbuf[a % 4, p, 0, rows, :], rbuf[a % 4, p, 1, rows, :])
                            for p in range(4)]) for a in (2 * r, 2 * r + 1)]
            for j in range(8):
                even = pltpu.bitcast(ys[0][j].astype(bf16).astype(f32), i32)
                odd = pltpu.bitcast(ys[1][j].astype(bf16).astype(f32), i32)
                yv[r, rows, j * 128:(j + 1) * 128] = lax.shift_right_logical(even, 16) | odd

    pending = {}
    for i in range(64 + 9):
        if i < 64:
            pending[i] = sequence_stage(*divmod(i, 4))
        if 1 <= i <= 64:
            feature_stage(*divmod(i - 1, 4), pending.pop(i - 1))
        if i >= 9:
            butterflies(*divmod(i - 9, 8))


def _interleave_heads(w, items, pieces=1):
    per_piece = D // 16 // pieces
    for first in range(0, D // 16, per_piece):
        for i in items:
            for c in range(first, first + per_piece, 2):
                even, odd = w[i, c:c + 2, 0], w[i, c:c + 2, 1]
                w[i, c:c + 2, 0] = (even & 0xFFFF) | (odd << 16)
                w[i, c:c + 2, 1] = lax.shift_right_logical(even, 16) | (odd & _HI16)
        yield


def _head_weight(w, i, e):
    return _halves(w[i, :, e].reshape(D // 2, DH))


def _segment(s, wqkv, wo32, xs, early_rows, h_ref, outs):
    z0 = pl.multiple_of(s * 8, 8)
    h_ref[M:L, :] = xs[s].astype(f32)
    row = lax.broadcasted_iota(i32, (L, L), 0)
    col = lax.broadcasted_iota(i32, (L, L), 1)
    mask = (row < M) | (row >= col)

    def project(h):
        items = [m * NPAIR + h // 2 for m in range(3)]
        ws = [_head_weight(wqkv, i, h % 2) for i in items]
        rows = [L - 8 if i < EARLY_ITEMS else L for i in items]
        if h == 0:
            first = [_dot(h_ref[0:n, 0:D // 2], w[0:D // 2]) for n, w in zip(rows, ws)]
            qkv = [_dot(h_ref[0:n, D // 2:D], w[D // 2:D]) + f for n, w, f in zip(rows, ws, first)]
        else:
            qkv = [_dot(h_ref[0:n, :], w) for n, w in zip(rows, ws)]
        return [jnp.concatenate([v, early_rows[2 * i + h % 2, pl.ds(z0, 8), :]], axis=0)
                if i < EARLY_ITEMS else v for v, i in zip(qkv, items)]

    def probabilities(q, k):
        sc = _dot(q, k.astype(bf16), _NT) * DH ** -0.5
        sc = jnp.where(mask, sc, -1e9)
        e = jnp.exp(sc - jnp.max(sc, axis=-1, keepdims=True))
        return e * pltpu.reciprocal(jnp.sum(e, axis=-1, keepdims=True), approx=False)

    def out_proj(o, n, lo, hi):
        w = _halves(wo32[n, lo * DH // 2:hi * DH // 2, :])
        return _dot(jnp.concatenate(o[lo:hi], axis=1), w)

    lag_scores, lag_mix, split = 2, 4, 24
    state, o, part = {}, [None] * H, [None] * 8
    for t in range(H + 8):
        if t < H:
            state[t] = project(t)
        else:
            part[t - H] = out_proj(o, t - H, 0, split)
        if 0 <= t - lag_scores < H:
            q, k, v = state[t - lag_scores]
            state[t - lag_scores] = (probabilities(q, k), v)
        if 0 <= t - lag_mix < H:
            p, v = state.pop(t - lag_mix)
            o[t - lag_mix] = _dot(p, v.astype(bf16))
    for n in range(8):
        res = out_proj(o, n, split, H) + part[n]
        h_ref[0:M, n * 128:(n + 1) * 128] = res[0:M]
        for i in range(SEG // 16):
            outs[2 * s + i, :, n * 128:(n + 1) * 128] = res[M + 16 * i:M + 16 * i + 16].astype(bf16)


def _kernel(ax_hbm, wr_hbm, wi_hbm, bx_hbm, mem0_hbm, wq_hbm, wk_hbm, wv_hbm, wo_hbm, out_hbm,
            xv, wrv, wiv, wnr, wni, m1, m2, gbuf, rbuf, yv,
            wqkv, wo, xs, xz_raw, xz, early_rows, mem0_ref, h_ref, outs,
            sem_ax, sem_f, sem_w, sem_wo, sem_bx, sem_xz, sem_ya, sem_yb):
    ax32 = ax_hbm.bitcast(i32)
    out32 = out_hbm.bitcast(i32)

    def ax_copy(r):
        return pltpu.make_async_copy(ax32.at[:, r, :], xv.at[r], sem_ax.at[r])

    def ya_copy(r):
        return pltpu.make_async_copy(yv.at[r], out32.at[:, r, pl.ds(0, D)], sem_ya.at[0])

    def bx_copy(c):
        return pltpu.make_async_copy(bx_hbm.at[pl.ds(c * SCHUNK, SCHUNK)],
                                     xs.at[pl.ds(c * SCHUNK, SCHUNK)], sem_bx.at[c])

    def yb_copy(c):
        rows = pl.ds(c * (SCHUNK * SEG // 16), SCHUNK * SEG // 16)
        return pltpu.make_async_copy(outs.at[rows], out_hbm.at[rows, :, pl.ds(D, D)], sem_yb.at[0])

    f_copies = [pltpu.make_async_copy(src.at[pl.ds(0, D // 2), pl.ds(k1 * 128, 128)],
                                      dst.at[k1, pl.ds(0, D // 4)].bitcast(bf16), sem_f.at[0])
                for k1 in range(16) for src, dst in ((wr_hbm, wrv), (wi_hbm, wiv))]
    f_copies += [pltpu.make_async_copy(src.at[pl.ds(D // 2, 1), :], dst, sem_f.at[0])
                 for src, dst in ((wr_hbm, wnr), (wi_hbm, wni))]
    wo_copies = [pltpu.make_async_copy(wo_hbm.at[:, pl.ds(n * 128, 128)], wo.at[n], sem_wo.at[0])
                 for n in range(8)]
    wo_copies.append(pltpu.make_async_copy(mem0_hbm, mem0_ref, sem_wo.at[0]))

    def start_pair(m, j):
        w32 = (wq_hbm, wk_hbm, wv_hbm)[m].bitcast(i32)
        for e in range(2):
            pltpu.make_async_copy(w32.at[:, :, e, j, :], wqkv.at[m * NPAIR + j, :, e],
                                  sem_w.at[m * NPAIR + j]).start()

    def wait_item(i):
        pltpu.make_async_copy(wqkv.at[i], wqkv.at[i], sem_w.at[i]).wait()

    for r in range(8):
        ax_copy(r).start()
    xz_copy = pltpu.make_async_copy(bx_hbm.at[:, pl.ds(SEG - 8, 8), :], xz_raw, sem_xz.at[0])
    xz_copy.start()
    for j in range(FIRST_ITEMS + 2):
        start_pair(0, j)
    for cp in f_copies:
        cp.start()

    _build_dft_matrices(m1, m2)
    m1, m2 = m1.bitcast(i32), m2.bitcast(i32)

    def wait_x(r):
        for i in {0: (0,), 1: (1, 2), 3: (3, 4, 5), 6: (6, 7)}.get(r, ()):
            ax_copy(i).wait()
        if r == 6:
            xz_copy.wait()
            for i in range(2):
                wait_item(i)

    def prepare_early():
        interleave = _interleave_heads(wqkv, (0, 1), 16)
        for c in range(0, NSEG, 4):
            xz[c * 8:(c + 4) * 8, :] = xz_raw[c:c + 4].astype(f32).reshape(32, D)
            next(interleave)
            yield

    _forward(xv, m1, m2, gbuf, wait_x, prepare_early())

    for j in range(FIRST_ITEMS + 2, NPAIR):
        start_pair(0, j)

    def filter_groups(t):
        for k1 in range(8):
            extract = (_lo_f32, _hi_f32)[k1 % 2]
            g = t + (16 * k1 if k1 < 4 else 16 * ((8 - k1) % 4) + 8)
            yield from _filter_rows(g, gbuf, lambda k: tuple(
                extract(w[k, pl.ds(32 * t + k1 // 2, 8, stride=4), :]) for w in (wrv, wiv)))

    def project_early(items, interleave_work, filter_work=iter(()), pieces=lambda n: 0):
        for n, (i, e, r0) in enumerate((i, e, r0) for i in items for e in range(2)
                                       for r0 in range(0, NSEG * 8, 64)):
            res = _dot(xz[r0:r0 + 64, :], _head_weight(wqkv, i, e))
            early_rows[2 * i + e, r0:r0 + 64, :] = res
            gbuf[65 + i % 2, 0, :, 0:128] = res[56:64]
            next(interleave_work, None)
            for _ in range(pieces(n)):
                next(filter_work, None)
        assert not list(interleave_work) and not list(filter_work)

    @pl.loop(0, FIRST_ITEMS // 2)
    def _(t):
        ahead = (2 * t + 2, 2 * t + 3)
        for i in ahead:
            wait_item(i)
        filter_work = (x for n in range(21) for x in _filter_rows(21 * t + n, gbuf))
        project_early((2 * t, 2 * t + 1), _interleave_heads(wqkv, ahead, 32),
                      filter_work, lambda n: 2 if n % 3 == 2 else 3)

    for g in range(63, 65):
        list(_filter_rows(g, gbuf))
    for j in range(NPAIR):
        start_pair(1, j)
    for cp in f_copies:
        cp.wait()

    @pl.loop(0, 4)
    def _(u):
        for i in range(4):
            start_pair(2, 4 * u + i)

        @pl.loop(2 * u, 2 * u + 2)
        def _(t):
            ahead = (FIRST_ITEMS + 2 * t + 2, FIRST_ITEMS + 2 * t + 3)
            for i in ahead:
                wait_item(i)
            project_early((FIRST_ITEMS + 2 * t, FIRST_ITEMS + 2 * t + 1),
                          _interleave_heads(wqkv, ahead, 32),
                          filter_groups(t), lambda n: 3 if n % 8 == 0 else 2)

    bx_copy(0).start()
    for cp in wo_copies:
        cp.start()
    list(_filter_rows(64, gbuf, lambda k: tuple(
        jnp.broadcast_to(w[:, k * 128:(k + 1) * 128].astype(f32), (8, 128)) for w in (wnr, wni))))

    _inverse(m1, m2, gbuf, rbuf, yv)

    done = FIRST_ITEMS + 16
    steps = (EARLY_ITEMS - done) // 2
    per_step = (3 * NPAIR - done - 2) // steps
    assert done + 2 * steps == EARLY_ITEMS and done + 2 + per_step * steps == 3 * NPAIR
    for i in range(done + 2, 3 * NPAIR):
        wait_item(i)

    @pl.loop(0, steps)
    def _(t):
        ahead = [done + 2 + per_step * t + i for i in range(per_step)]
        project_early((done + 2 * t, done + 2 * t + 1), _interleave_heads(wqkv, ahead, 32))

    for cp in wo_copies:
        cp.wait()
    for c in range(1, NCHUNK):
        bx_copy(c).start()
    for r in range(8):
        ya_copy(r).start()
    h_ref[0:M, :] = mem0_ref[...].astype(f32)
    wo32 = wo.bitcast(i32)

    @pl.loop(0, NCHUNK)
    def _(c):
        bx_copy(c).wait()
        for i in range(SCHUNK):
            _segment(c * SCHUNK + i, wqkv, wo32, xs, early_rows, h_ref, outs)
        yb_copy(c).start()

    for r in range(8):
        ya_copy(r).wait()
    for c in range(NCHUNK):
        yb_copy(c).wait()


@functools.partial(jax.jit, static_argnames=("B_seg_len",))
def pallas_concat_heads__spectral_gfnet__memory_aug_recurrent_mem_tr__prompt_kernel(
    A_x, A_w_r, A_w_i, B_x, B_mem0, B_Wq, B_Wk, B_Wv, B_Wo, B_seg_len,
):
    assert A_x.shape == (1, S, D) and B_x.shape == (1, S, D) and B_mem0.shape == (1, M, D)
    assert A_w_r.shape == (S, D // 2 + 1) and B_Wq.shape == (D, H, DH) and B_Wo.shape == (H, DH, D)
    assert B_seg_len == SEG
    hbm = pl.BlockSpec(memory_space=pl.ANY)
    out = pl.pallas_call(
        _kernel,
        out_shape=jax.ShapeDtypeStruct((S // 16, 16, 2 * D), bf16),
        in_specs=[hbm] * 9,
        out_specs=hbm,
        scratch_shapes=[
            pltpu.VMEM((8, 128, D), i32),
            pltpu.VMEM((16, D // 4 + 8, 128), i32),
            pltpu.VMEM((16, D // 4 + 8, 128), i32),
            pltpu.VMEM((1, S), bf16),
            pltpu.VMEM((1, S), bf16),
            pltpu.VMEM((4, 3, 128, 128), bf16),
            pltpu.VMEM((16, 3, 128, 128), bf16),
            pltpu.VMEM((67, 16, 8, 256), f32),
            pltpu.VMEM((4, 4, 2, 128, 128), f32),
            pltpu.VMEM((8, 128, D), i32),
            pltpu.VMEM((3 * NPAIR, D // 16, 2, 8, DH), i32),
            pltpu.VMEM((8, H * DH, 128), bf16),
            pltpu.VMEM((NSEG, SEG, D), bf16),
            pltpu.VMEM((NSEG, 8, D), bf16),
            pltpu.VMEM((NSEG * 8, D), f32),
            pltpu.VMEM((2 * EARLY_ITEMS, NSEG * 8, DH), f32),
            pltpu.VMEM((M, D), bf16),
            pltpu.VMEM((L, D), f32),
            pltpu.VMEM((S // 16, 16, D), bf16),
            pltpu.SemaphoreType.DMA((8,)),
            pltpu.SemaphoreType.DMA((1,)),
            pltpu.SemaphoreType.DMA((3 * NPAIR,)),
            pltpu.SemaphoreType.DMA((1,)),
            pltpu.SemaphoreType.DMA((NCHUNK,)),
            pltpu.SemaphoreType.DMA((1,)),
            pltpu.SemaphoreType.DMA((1,)),
            pltpu.SemaphoreType.DMA((1,)),
        ],
        compiler_params=pltpu.CompilerParams(vmem_limit_bytes=100 * 1024 * 1024),
    )(
        A_x.reshape(S // 16, 16, D), A_w_r.T, A_w_i.T,
        B_x.reshape(NSEG, SEG, D), B_mem0.reshape(M, D),
        B_Wq.reshape(D // 16, 8, 2, H, DH), B_Wk.reshape(D // 16, 8, 2, H, DH),
        B_Wv.reshape(D // 16, 8, 2, H, DH), B_Wo.reshape(H * DH, D),
    )
    return out.reshape(1, S, 2 * D)
```
